```python
import jax
import jax.numpy as jnp

def _softmax(x, axis=-1):
    return jax.nn.softmax(x, axis=axis)
def _gelu(x):
    return jax.nn.gelu(x, approximate=True)
def _silu(x):
    return jax.nn.silu(x)
def _sigmoid(x):
    return jax.nn.sigmoid(x)
def _layernorm(x, axis=-1, eps=1e-5):
    m = jnp.mean(x, axis=axis, keepdims=True)
    v = jnp.var(x, axis=axis, keepdims=True)
    return (x - m) / jnp.sqrt(v + eps)
def _scatter_add(tgt, idx, src, axis=0):
    return tgt.at[idx].add(src)
def _segment_sum(src, seg, n):
    return jax.ops.segment_sum(src, seg, n)
class _Rng:
    def __init__(self, key):
        self._k = key
    def _next(self):
        self._k, sub = jax.random.split(self._k)
        return sub
    def normal(self, shape):
        return jax.random.normal(self._next(), shape, dtype=jnp.bfloat16)
    def randint(self, lo, hi, shape):
        return jax.random.randint(self._next(), shape, lo, hi, dtype=jnp.int32)
    def uniform(self, shape, lo=0.0, hi=1.0):
        return jax.random.uniform(self._next(), shape, jnp.bfloat16, lo, hi)
    def permutation(self, n):
        return jax.random.permutation(self._next(), n)


kernel_name = 'concat_heads__linear_attn_block__ssm_conv_h3__prompt'

def setup_inputs():
    _rng = _Rng(jax.random.key(int.from_bytes(__import__("os").urandom(4), "little")))
    _w = (lambda a: (lambda t: t.astype(jnp.bfloat16) if jnp.issubdtype(t.dtype, jnp.floating) else t)(jnp.asarray(a)))
    def _A_setup():
        B, S, D = 1, 2048, 1024
        return {
            "x": _w((lambda *s: _rng.normal(s) * 0.05)(B, S, D)),
            "wqkv": _w((lambda *s: _rng.normal(s) * 0.05)(D, 3 * D)),
            "wo": _w((lambda *s: _rng.normal(s) * 0.05)(D, D)),
        }
    _A_in = _A_setup()

    def _B_setup():
        B, S, D = 1, 2048, 1024
        ks = 4
        return {
            "q": _w((lambda *s: _rng.normal(s) * 0.05)(B, S, D)),
            "k": _w((lambda *s: _rng.normal(s) * 0.05)(B, S, D)),
            "v": _w((lambda *s: _rng.normal(s) * 0.05)(B, S, D)),
            "shift_k": _w((lambda *s: _rng.normal(s) * 0.05)(D, ks) * 0.5),
            "ssm_k": _w((lambda *s: _rng.normal(s) * 0.05)(D, S) * (1.0 / S ** 0.5)),
            "ssm_D": _w((lambda *s: _rng.normal(s) * 0.05)(D)),
        }
    _B_in = _B_setup()

    return {
        "A_x": _A_in["x"],
        "A_wqkv": _A_in["wqkv"],
        "A_wo": _A_in["wo"],
        "B_q": _B_in["q"],
        "B_k": _B_in["k"],
        "B_v": _B_in["v"],
        "B_shift_k": _B_in["shift_k"],
        "B_ssm_k": _B_in["ssm_k"],
        "B_ssm_D": _B_in["ssm_D"],
    }

def reference(A_x, A_wqkv, A_wo, B_q, B_k, B_v, B_shift_k, B_ssm_k, B_ssm_D):
    def _A_ref(x, wqkv, wo):
        B, S, D = x.shape
        H = 32; Dh = D // H
        qkv = (lambda x, *d: x.transpose(*d))((x @ wqkv).reshape(B, S, 3, H, Dh), 2, 0, 3, 1, 4)
        q, k, v = qkv[0], qkv[1], qkv[2]
        phi = lambda t: jnp.where(t > 0, t + 1, jnp.exp(t)) + 1e-6
        pq, pk = phi(q), phi(k)
        kv = jnp.einsum("bhsd,bhse->bhde", pk, v)
        z = jnp.einsum("bhsd->bhd", pk)
        num = jnp.einsum("bhqd,bhde->bhqe", pq, kv)
        den = jnp.einsum("bhqd,bhd->bhq", pq, z)[..., None] + 1e-6
        o = num / den
        return (lambda x, *d: x.transpose(*d))(o, 0, 2, 1, 3).reshape(B, S, D) @ wo

    def _B_ref(q, k, v, shift_k, ssm_k, ssm_D):
        B, S, D = q.shape
        ks = shift_k.shape[-1]
        k_pad = jnp.pad(k, ((0, 0), (ks - 1, 0), (0, 0)))
        k_shift = jnp.zeros_like(k)
        for t in range(ks):
            k_shift = k_shift + k_pad[:, t:t + S, :] * shift_k[:, ks - 1 - t][None, None, :]
        kv = k_shift * v
        L = 2 * S
        kv_pad = jnp.pad(kv, ((0, 0), (0, S), (0, 0)))
        kf_pad = jnp.pad(ssm_k, ((0, 0), (0, S)))
        kv_f = (lambda x, axes=(-2,-1): jnp.fft.rfft2(x.astype(jnp.float32), axes=axes))(kv_pad[:, None, :, :], axes=(1, 2))
        kf_f = (lambda x, axes=(-2,-1): jnp.fft.rfft2(x.astype(jnp.float32), axes=axes))(kf_pad[:, None, :], axes=(1, 2))
        kf_f = (lambda x, *d: x.transpose(*d))(kf_f, 1, 2, 0)
        y_f = kv_f * kf_f[None, :, :, :]
        y = (lambda x, s, axes=(-2,-1): jnp.fft.irfft2(x, s=s, axes=axes).astype(jnp.bfloat16))(y_f, (1, L), axes=(1, 2))[:, 0, :S, :]
        y = y + kv * ssm_D[None, None, :]
        return q * y

    a = _A_ref(A_x, A_wqkv, A_wo)
    b = _B_ref(B_q, B_k, B_v, B_shift_k, B_ssm_k, B_ssm_D)
    return jnp.concatenate([a, b], axis=-1)
```

```python
import functools

import jax
import jax.numpy as jnp
import numpy as np
from jax import lax
import jax.experimental.pallas as pl
import jax.experimental.pallas.tpu as pltpu

BF = jnp.bfloat16
F32 = jnp.float32
S = 2048
D = 1024
C = 128
NC = S // C
NB = D // C
DH = 32


def _dft_matrix():
    n = np.arange(C, dtype=np.float64)[None, :]
    m = np.arange(C, dtype=np.float64)[:, None]
    theta = 2.0 * np.pi * (m + 0.25) / C
    return np.concatenate([np.cos(theta * n), -np.sin(theta * n)], axis=0)


_F = _dft_matrix()
_FWD = _F.astype(np.float32)
_INV = (_F.T / C).astype(np.float32)

NT = (((1,), (1,)), ((), ()))
TN = (((0,), (0,)), ((), ()))


def _phi(t):
    return jnp.where(t > 0, t + 1.0, jnp.exp(t)) + 1e-6


def _kernel(x_hbm, w_hbm, wo_hbm, q_hbm, k_hbm, v_hbm, sk_hbm, shift_ref, d_ref, f_ref, fi_ref,
            o_hbm,
            x_v, w_v, wo_v, q_v, k_v, v_v, sk_v, ob_v, oa_v,
            kf_s, uh_s, kh_s, yh_s, pq_s, op_s, m_s, par_s,
            sem_x, sem_in, sem_o, *, R, R2, U1, U2, U3):
    NX = 4
    XR = S // NX

    def x_copy(c):
        rows = pl.ds(c * XR, XR)
        return pltpu.make_async_copy(x_hbm.at[rows, :], x_v.at[rows, :], sem_x.at[c])

    def in_copies(i):
        cols = pl.ds(pl.multiple_of(i * C, C), C)
        cps = [
            pltpu.make_async_copy(k_hbm.at[:, cols], k_v.at[i], sem_in.at[0, i]),
            pltpu.make_async_copy(v_hbm.at[:, cols], v_v.at[i], sem_in.at[1, i]),
            pltpu.make_async_copy(sk_hbm.at[cols, :], sk_v.at[i], sem_in.at[2, i]),
        ]
        for t in range(3):
            wc = pl.ds(pl.multiple_of(t * D + i * C, C), C)
            cps.append(pltpu.make_async_copy(w_hbm.at[:, wc], w_v.at[i, t], sem_in.at[3 + t, i]))
        cps.append(pltpu.make_async_copy(q_hbm.at[:, cols], q_v.at[i], sem_in.at[6, i]))
        cps.append(pltpu.make_async_copy(wo_hbm.at[cols, :], wo_v.at[i], sem_in.at[7, i]))
        return cps

    def ob_copy(i):
        cols = pl.ds(pl.multiple_of(D + i * C, C), C)
        return pltpu.make_async_copy(ob_v.at[i], o_hbm.at[:, cols], sem_o.at[i])

    def oa_copy(r):
        rows = pl.ds(pl.multiple_of(r * R2, R2), R2)
        return pltpu.make_async_copy(oa_v.at[rows, :], o_hbm.at[rows, pl.ds(0, D)], sem_o.at[NB + r])

    first = in_copies(0)
    for cp in first[:6]:
        cp.start()
    for c in range(NX):
        x_copy(c).start()
    for cp in first[6:]:
        cp.start()

    sh = shift_ref[...].astype(F32)
    dd = d_ref[...].astype(F32).reshape(1, D)
    for i in range(NB):
        par_s[i, 0:4, :] = sh[:, i * C:(i + 1) * C]
        par_s[i, 4:5, :] = dd[:, i * C:(i + 1) * C]
    kf_s[0:8, :] = jnp.zeros((8, C), F32)

    row_h = lax.broadcasted_iota(jnp.int32, (C, C), 0) // DH
    col_h = lax.broadcasted_iota(jnp.int32, (C, C), 1) // DH
    same_head = row_h == col_h

    def step(i, carry):
        cps = in_copies(i)

        @pl.when(i + 1 < NB)
        def _():
            for cp in in_copies(i + 1):
                cp.start()

        for cp in cps[:3]:
            cp.wait()

        taps = [jnp.broadcast_to(par_s[i, j:j + 1, :], (C, C)) for j in range(4)]

        def fwd(a, c):
            r0 = pl.multiple_of(a * C, C)
            rows = pl.ds(r0, C)
            kk = k_v[i, rows, :].astype(F32)
            kf_s[pl.ds(r0 + 8, C), :] = kk
            ks = kk * taps[0]
            for j in range(1, 4):
                ks = ks + kf_s[pl.ds(r0 + 8 - j, C), :] * taps[j]
            u = (ks * v_v[i, rows, :].astype(F32)).astype(BF)
            uh_s[a] = jnp.dot(f_ref[...], u, preferred_element_type=F32)
            kh_s[a] = lax.dot_general(f_ref[...], sk_v[i, :, rows], NT, preferred_element_type=F32)
            return c

        lax.fori_loop(0, NC, fwd, 0, unroll=U1)

        for cp in cps[3:6]:
            cp.wait()

        @pl.when(i == 0)
        def _():
            for c in range(NX):
                x_copy(c).wait()

        skip = jnp.broadcast_to(par_s[i, 4:5, :], (8, C))

        def freq_conv(f0):
            re = pl.ds(f0, 8)
            im = pl.ds(C + f0, 8)
            cs = [kh_s[j, re, :] for j in range(NC)]
            ds_ = [kh_s[j, im, :] for j in range(NC)]
            cs[0] = cs[0] + skip
            c2 = [cs[0]] + [cs[j] - ds_[j - 1] for j in range(1, NC)]
            d2 = [ds_[0]] + [ds_[j] + cs[j - 1] for j in range(1, NC)]
            ua = [uh_s[j, re, :] for j in range(NC)]
            ub = [uh_s[j, im, :] for j in range(NC)]

            def conv(p, q):
                out = []
                for a in range(NC):
                    acc = p[0] * q[a]
                    for j in range(1, a + 1):
                        acc = acc + p[j] * q[a - j]
                    out.append(acc)
                return out

            s1 = conv(c2, [ua[j] + ub[j] for j in range(NC)])
            s2 = conv([d2[j] - c2[j] for j in range(NC)], ua)
            s3 = conv([d2[j] + c2[j] for j in range(NC)], ub)
            return [s1[a] - s3[a] for a in range(NC)], [s1[a] + s2[a] for a in range(NC)]

        NR = S // R
        FG = C // NR

        def main(j, c):
            kv, z = c
            rows = pl.ds(pl.multiple_of(j * R, R), R)
            w = jnp.concatenate([w_v[i, t] for t in range(3)], axis=1)
            qkv = jnp.dot(x_v[rows, :], w, preferred_element_type=F32)
            pq_s[rows, :] = _phi(qkv[:, 0:C])
            pk = _phi(qkv[:, C:2 * C])
            z = z + jnp.sum(pk.reshape(R // 8, 8, C), axis=0)
            kv = kv + lax.dot_general(pk.astype(BF), qkv[:, 2 * C:].astype(BF), TN, preferred_element_type=F32)
            for g in range(FG // 16):
                f0 = pl.multiple_of(j * FG + g * 16, 16)
                ra, ia = freq_conv(f0)
                rb, ib = freq_conv(f0 + 8)
                for a in range(NC):
                    yh_s[a, pl.ds(f0, 16), :] = jnp.concatenate([ra[a], rb[a]], axis=0).astype(BF)
                    yh_s[a, pl.ds(C + f0, 16), :] = jnp.concatenate([ia[a], ib[a]], axis=0).astype(BF)
            return kv, z

        kv, z = lax.fori_loop(0, NR, main, (jnp.zeros((C, C), F32), jnp.zeros((8, C), F32)), unroll=U2)

        for cp in cps[6:]:
            cp.wait()

        zrow = jnp.sum(z, axis=0, keepdims=True)
        zt = jnp.where(same_head, jnp.broadcast_to(zrow, (C, C)), 0.0).astype(BF)
        kvb = jnp.where(same_head, kv, 0.0).astype(BF)
        m_s[pl.ds(pl.multiple_of(i * C, C), C), :] = jnp.dot(kvb, wo_v[i], preferred_element_type=F32).astype(BF)

        def tail(a, c):
            rows = pl.ds(pl.multiple_of(a * C, C), C)
            y = jnp.dot(fi_ref[...], yh_s[a], preferred_element_type=F32)
            ob_v[i, rows, :] = (y * q_v[i, rows, :].astype(F32)).astype(BF)
            pq = pq_s[rows, :]
            den = lax.dot_general(pq.astype(BF), zt, NT, preferred_element_type=F32) + 1e-6
            op_s[i, rows, :] = (pq / den).astype(BF)
            return c

        lax.fori_loop(0, NC, tail, 0, unroll=U3)
        ob_copy(i).start()
        return carry

    lax.fori_loop(0, NB, step, 0)

    def proj(r, c):
        rows = pl.ds(pl.multiple_of(r * R2, R2), R2)
        o = jnp.concatenate([op_s[t, rows, :] for t in range(NB)], axis=1)
        oa_v[rows, :] = jnp.dot(o, m_s[...], preferred_element_type=F32).astype(BF)
        oa_copy(r).start()
        return c

    lax.fori_loop(0, S // R2, proj, 0)
    for i in range(NB):
        ob_copy(i).wait()
    for r in range(S // R2):
        oa_copy(r).wait()


def make(R=256, R2=256, U1=4, U2=1, U3=4):
    @jax.jit
    def fn(A_x, A_wqkv, A_wo, B_q, B_k, B_v, B_shift_k, B_ssm_k, B_ssm_D):
        hbm = pl.BlockSpec(memory_space=pl.ANY)
        vmem = pl.BlockSpec(memory_space=pltpu.VMEM)
        out = pl.pallas_call(
            functools.partial(_kernel, R=R, R2=R2, U1=U1, U2=U2, U3=U3),
            out_shape=jax.ShapeDtypeStruct((S, 2 * D), BF),
            in_specs=[hbm] * 7 + [vmem] * 4,
            out_specs=hbm,
            scratch_shapes=[
                pltpu.VMEM((S, D), BF),
                pltpu.VMEM((NB, 3, D, C), BF),
                pltpu.VMEM((NB, C, D), BF),
                pltpu.VMEM((NB, S, C), BF),
                pltpu.VMEM((NB, S, C), BF),
                pltpu.VMEM((NB, S, C), BF),
                pltpu.VMEM((NB, C, S), BF),
                pltpu.VMEM((NB, S, C), BF),
                pltpu.VMEM((S, D), BF),
                pltpu.VMEM((S + 8, C), F32),
                pltpu.VMEM((NC, 2 * C, C), F32),
                pltpu.VMEM((NC, 2 * C, C), F32),
                pltpu.VMEM((NC, 2 * C, C), BF),
                pltpu.VMEM((S, C), F32),
                pltpu.VMEM((NB, S, C), BF),
                pltpu.VMEM((D, D), BF),
                pltpu.VMEM((NB, 8, C), F32),
                pltpu.SemaphoreType.DMA((4,)),
                pltpu.SemaphoreType.DMA((8, NB)),
                pltpu.SemaphoreType.DMA((NB + S // R2,)),
            ],
            compiler_params=pltpu.CompilerParams(vmem_limit_bytes=100 * 2**20),
        )(
            A_x.reshape(S, D), A_wqkv, A_wo,
            B_q.reshape(S, D), B_k.reshape(S, D), B_v.reshape(S, D),
            B_ssm_k, B_shift_k.T, B_ssm_D,
            jnp.asarray(_FWD, BF), jnp.asarray(_INV, BF),
        )
        return out.reshape(1, S, 2 * D)
    return fn


_fn = make(R=256,U1=16,U2=8,U3=16)


@jax.jit
def pallas_concat_heads__linear_attn_block__ssm_conv_h3__prompt_kernel(
    A_x: jax.Array,
    A_wqkv: jax.Array,
    A_wo: jax.Array,
    B_q: jax.Array,
    B_k: jax.Array,
    B_v: jax.Array,
    B_shift_k: jax.Array,
    B_ssm_k: jax.Array,
    B_ssm_D: jax.Array,
):
    return _fn(A_x, A_wqkv, A_wo, B_q, B_k, B_v, B_shift_k, B_ssm_k, B_ssm_D)
```

```python
import functools

import jax
import jax.numpy as jnp
import numpy as np
from jax import lax
import jax.experimental.pallas as pl
import jax.experimental.pallas.tpu as pltpu

BF = jnp.bfloat16
F32 = jnp.float32
S = 2048
D = 1024
C = 128
H = C // 2
NC = S // C
NB = D // C
NS = NB // 2
NJ = NC // 2
NG = NJ // 2
DH = 32

PIN = 28 * 8
UH = PIN + 16
KH = UH + 2 * NC * 2 * C
PACE_ROWS = KH + 2 * NC * 2 * C

T_ORDER = (1, 2, 0)
P_ORDER = (0, 5, 6, 1, 3, 4, 2)
NT = (((1,), (1,)), ((), ()))


def _dft_matrix():
    n = np.arange(C, dtype=np.float64)[None, :]
    m = np.arange(C, dtype=np.float64)[:, None]
    theta = 2.0 * np.pi * (m + 0.25) / C
    return np.concatenate([np.cos(theta * n), -np.sin(theta * n)], axis=0)


def _paired(n):
    pos = np.arange(n)
    return pos // 16 * 16 + pos % 2 * 8 + pos % 16 // 2


_FWD = np.stack([_dft_matrix(), _dft_matrix()[:, _paired(C)]]).astype(np.float32)
_INV = (_dft_matrix().T / C)[:, _paired(2 * C)].astype(np.float32)


def _phi(t):
    return jnp.where(t > 0, t + 1.0, jnp.exp(t)) + 1e-6


def _tree_sum(terms):
    while len(terms) > 1:
        terms = [terms[e] + terms[e + 1] if e + 1 < len(terms) else terms[e]
                 for e in range(0, len(terms), 2)]
    return terms[0]


def _pack_rows(even, odd):
    return pltpu.bitcast(pltpu.pack_elementwise([even, odd], packed_dtype=BF), F32)


class _Tile:
    def __init__(self, tile):
        bits = pltpu.bitcast(tile, jnp.uint32)
        self.words = pltpu.bitcast(bits, F32)
        self.even = pltpu.bitcast(bits << 16, F32)
        self.odd = pltpu.bitcast(bits & np.uint32(0xFFFF0000), F32)

    def __add__(self, other):
        return _pack_rows(self.even + other.even, self.odd + other.odd)

    def __sub__(self, other):
        return _pack_rows(self.even - other.even, self.odd - other.odd)


def _left_operands(*tiles):
    a11, a12, a21, a22 = (_Tile(t) for t in tiles)
    return [a11 + a22, a21 + a22, a11.words, a22.words, a11 + a12, a21 - a11, a12 - a22]


def _right_operands(*tiles):
    b11, b12, b21, b22 = (_Tile(t) for t in tiles)
    return [b11 + b22, b11.words, b12 - b22, b21 - b11, b22.words, b11 + b12, b21 + b22]


def _strassen(product, emit, fillers):
    def run(p):
        r = product(p)
        filler = fillers.pop(0)
        if filler is not None:
            filler()
        return r
    m = run(0)
    c11, c22 = m, m
    c22 = c22 + run(5)
    c11 = c11 + run(6)
    m = run(1)
    c21, c22 = m, c22 - m
    m = run(3)
    emit(1, 0, c21 + m)
    c11 = c11 + m
    m = run(4)
    emit(0, 0, c11 - m)
    c12 = m
    m = run(2)
    emit(0, 1, c12 + m)
    emit(1, 1, c22 + m)


class Background:
    def __init__(self, tasks, slots):
        self.tasks = [t for t, _ in tasks]
        self.left = [n for _, n in tasks]
        self.total = list(self.left)
        self.slots = slots
        self.slot = 0

    def advance(self):
        self.slot += 1
        for e, task in enumerate(self.tasks):
            keep = self.total[e] - min(self.total[e], -(-self.total[e] * self.slot // self.slots))
            while self.left[e] > keep:
                yield next(task)
                self.left[e] -= 1


def _kernel(zero_ref, x_hbm, w_hbm, wo_hbm, q_hbm, k_hbm, v_hbm, sk_hbm, shift_ref, d_ref, f_ref, fi_ref,
            o_hbm,
            pace0, pace1, xs_s, ws0, ws1, yh0, yh1, kf_s, us_s, tm_s, ms_s, os_s, x_v, w_v, wo_v, q_v, k_v, v_v, sk_v, ob_v, oa_v,
            pq_s, pkt_s, vv_s, kv_s, z_s, kvb_s, zt_s, op_s, m_s, par_s,
            sem_x, sem_c, sem_w, sem_t, sem_o, *, SLACK, POS, GS, GF, GO, LAG, REV, POS2, START1, UN):

    def aligned(start, size):
        return pl.ds(start if isinstance(start, int) else pl.multiple_of(start, size), size)

    pace, ws, yh = (pace0, pace1), (ws0, ws1), (yh0, yh1)

    def halves(tile):
        return pltpu.bitcast(tile, BF)

    def x_copies(g):
        cps = []
        for h in range(2):
            rows = aligned((2 * g + NJ * h) * C, 2 * C)
            cps += [pltpu.make_async_copy(x_hbm.at[rows, pl.ds(kt * C, C)], x_v.at[kt, rows, :], sem_x.at[g])
                    for kt in range(NB)]
        return cps

    def conv_in_copies(s, g, parts):
        span = aligned(g * (S // parts), S // parts)
        cps = []
        for i in (2 * s, 2 * s + 1):
            cols = pl.ds(i * C, C)
            cps += [pltpu.make_async_copy(k_hbm.at[span, cols], k_v.at[i, span, :], sem_c.at[s, g]),
                    pltpu.make_async_copy(v_hbm.at[span, cols], v_v.at[i, span, :], sem_c.at[s, g]),
                    pltpu.make_async_copy(sk_hbm.at[cols, span], sk_v.at[i, :, span], sem_c.at[s, g])]
        return cps

    def w_copies(s, g, parts, ts=T_ORDER):
        cps = []
        for half in range(2):
            rows = aligned(half * (D // 2) + g * (D // 2 // parts), D // 2 // parts)
            cps += [pltpu.make_async_copy(w_hbm.at[rows, pl.ds(t * D + i * C, C)], w_v.at[i, t, rows, :],
                                          sem_w.at[s, g + (t if len(ts) == 1 else 0)])
                    for t in ts for i in (2 * s, 2 * s + 1)]
        return cps

    def first_group(g):
        return x_copies(g) + conv_in_copies(0, g, NG) + w_copies(1, g, NG)

    def wo_copies(s):
        return [pltpu.make_async_copy(wo_hbm.at[pl.ds(s * 2 * C, 2 * C), :], wo_v.at[s], sem_t.at[0, s])]

    def q_copies(s):
        return [pltpu.make_async_copy(q_hbm.at[:, pl.ds(i * C, C)], q_v.at[i], sem_t.at[1, s])
                for i in (2 * s, 2 * s + 1)]

    def inputs_of(s):
        cps = wo_copies(s - 1)
        if s < NS:
            cps += conv_in_copies(s, 0, 1)
        if s + 1 < NS:
            cps += w_copies(s + 1, 0, 1)
        if s >= 2:
            cps += q_copies(s - 2)
        return cps

    def ob_copies(s, g=0, parts=1):
        rows = aligned(g * (S // parts), S // parts)
        return [pltpu.make_async_copy(ob_v.at[i, rows, :], o_hbm.at[rows, pl.ds(D + i * C, C)], sem_o.at[0, s + g])
                for i in (2 * s, 2 * s + 1)]

    def oa_copies(j):
        return [pltpu.make_async_copy(oa_v.at[j, h], o_hbm.at[aligned((j + NJ * h) * C, C), pl.ds(0, D)],
                                      sem_o.at[1 + h, j]) for h in range(2)]

    def start(cps):
        for cp in cps:
            cp.start()

    def wait(cps):
        for cp in cps:
            cp.wait()

    def short_conv_task(s, j):
        for b in range(2):
            i = 2 * s + b
            taps = [jnp.broadcast_to(par_s[i, e:e + 1, :], (8, C)) for e in range(4)]
            for c in range(2):
                r0 = (2 * j + c) * C
                kf_s[b, pl.ds(pl.multiple_of(r0 + 8, 8), C), :] = k_v[i, aligned(r0, C), :].astype(F32)
                for r1 in range(0, C, GS):
                    vv = v_v[i, aligned(r0 + r1, GS), :].astype(F32)
                    parts = []
                    for r in range(0, GS, 8):
                        ks = _tree_sum([kf_s[b, pl.ds(r0 + r1 + r + 8 - e, 8), :] * taps[e] for e in range(4)])
                        parts.append(ks * vv[r:r + 8])
                    us_s[2 * b + c, r1 // 2:(r1 + GS) // 2, :] = jnp.concatenate(
                        [_pack_rows(*parts[e:e + 2]) for e in range(0, len(parts), 2)], axis=0)
                    yield parts[-1]
    SHORT_STEPS = 4 * (C // GS)

    def freq_conv_task(s, j):
        src = pace[(s + 1) % 2]
        for b in range(2):
            skip = jnp.broadcast_to(par_s[2 * s + b, 4:5, :], (8, C))
            for t in range(3):
                for h in range(2):
                    def parts(base, a):
                        row = base + (b * NC + a) * 2 * C + j * 16 + 8 * h
                        return (lambda: src[aligned(row, 8), :]), (lambda: src[aligned(row + C, 8), :])

                    p, q, before = [], [], None
                    for a in range(NC):
                        if a == 0 or a in GF:
                            for e in range(a, min(g for g in GF if g > a)):
                                kr, ki = parts(KH, e)
                                ur, ui = parts(UH, e)
                                kr = kr() + skip if e == 0 else kr()
                                p.append(kr if t == 0 else ki() - kr if t == 1 else ki() + kr)
                                q.append(ur() + ui() if t == 0 else ur() if t == 1 else ui())
                        acc = _tree_sum([p[e] * q[a - e] for e in range(a + 1)])
                        if t == 0:
                            tm_s[b, h, a] = acc
                        elif t == 1:
                            acc = tm_s[b, h, a] + acc
                            tm_s[b, 2 + h, a] = acc
                        else:
                            re, im = tm_s[b, h, a] - acc, tm_s[b, 2 + h, a]
                            yr, yi = (re, im) if a == 0 else (re - before[1], im + before[0])
                            before, acc = (re, im), yr
                            if h == 0:
                                tm_s[b, 4, a] = yr
                                tm_s[b, 5, a] = yi
                            else:
                                yh[s % 2][b, a, aligned(j * 8, 8), :] = _pack_rows(tm_s[b, 4, a], yr)
                                yh[s % 2][b, a, aligned(H + j * 8, 8), :] = _pack_rows(tm_s[b, 5, a], yi)
                        if a + 1 in GF:
                            yield acc
    FREQ_STEPS = 2 * 3 * 2 * len(GF)

    def w_operand_task(s, j, ts=T_ORDER):
        for t in ts:
            top, bot = aligned(j * 64, 64), aligned(D // 2 + j * 64, 64)
            ops = _right_operands(w_v[2 * s, t, top, :], w_v[2 * s + 1, t, top, :],
                                  w_v[2 * s, t, bot, :], w_v[2 * s + 1, t, bot, :])
            for p in range(7):
                ws[s % 2][t, p, aligned(j * 32, 32), :] = ops[p]
            yield ops[6][:8]
    W_STEPS = 3

    def publish_heads(dst, src, order):
        for e, t in enumerate(order):
            for g, p in enumerate(P_ORDER):
                dst[pl.ds((e * 7 + g) * 8, 8), :] = src[t, p, 0:8, :]

    def left_operand_task(src, dst, j):
        for kt in range(4):
            for r in range(0, C, GO):
                top, bot = aligned(j * C + r, GO), aligned((j + NJ) * C + r, GO)
                ops = _left_operands(src[kt, top, :], src[4 + kt, top, :], src[kt, bot, :], src[4 + kt, bot, :])
                for p in range(7):
                    dst[p, kt, r // 2:(r + GO) // 2, :] = ops[p]
                yield ops[6][:8]
    LEFT_STEPS = 4 * (C // GO)

    def run(task):
        for _ in task:
            pass

    def m_operands(n):
        for kt in range(4):
            top, bot = pl.ds(kt * C, C), pl.ds(D // 2 + kt * C, C)
            ops = _right_operands(m_s[n, top, :], m_s[4 + n, top, :], m_s[n, bot, :], m_s[4 + n, bot, :])
            for p in range(7):
                ms_s[n, p, pl.ds(kt * H, H), :] = ops[p]

    def store_spectra(s, j, base, spec):
        for b in range(2):
            for c in range(2):
                row = pl.multiple_of(base + (b * NC + 2 * j + c) * 2 * C, 8)
                pace[(s + 1) % 2][pl.ds(row, 2 * C), :] = spec[:, (2 * b + c) * C:(2 * b + c + 1) * C]

    def kernel_spectra(s, j):
        taps = jnp.concatenate([sk_v[2 * s + b, :, aligned((2 * j + c) * C, C)] for b in range(2) for c in range(2)],
                               axis=0)
        spec = lax.dot_general(f_ref[0], taps, NT, preferred_element_type=F32)
        store_spectra(s, j, KH, spec)

    def input_spectra(s, j):
        u = jnp.concatenate([halves(us_s[e]) for e in range(4)], axis=1)
        spec = jnp.dot(f_ref[1], u, preferred_element_type=F32)
        store_spectra(s, j, UH, spec)

    def conv_output(s, j, b):
        i = 2 * s + b
        spec = jnp.concatenate([pltpu.bitcast(yh[s % 2][b, 2 * j + c], BF) for c in range(2)], axis=1)
        y = jnp.dot(fi_ref[...], spec, preferred_element_type=F32)
        for c in range(2):
            rows = aligned((2 * j + c) * C, C)
            ob_v[i, rows, :] = (y[:, c * C:(c + 1) * C] * q_v[i, rows, :].astype(F32)).astype(BF)

    def normalise(s, b, a):
        rows = aligned(a * C, C)
        pq = pq_s[s % 2, b, rows, :]
        den = lax.dot_general(pq.astype(BF), zt_s[b], NT, preferred_element_type=F32) + 1e-6
        r = pl.reciprocal(den, approx=True)
        r = r * (2.0 - den * r)
        op_s[2 * s + b, rows, :] = (pq * r).astype(BF)

    def fold_wo(s, b, n):
        wo = wo_v[s, pl.ds(b * C, C), aligned(n * C, C)]
        m_s[n, aligned((2 * s + b) * C, C), :] = jnp.dot(kvb_s[b], wo, preferred_element_type=F32).astype(BF)

    def finish_state():
        same_head = (lax.broadcasted_iota(jnp.int32, (C, C), 0) // DH
                     == lax.broadcasted_iota(jnp.int32, (C, C), 1) // DH)
        for b in range(2):
            z = jnp.sum(z_s[b], axis=0, keepdims=True)
            zt_s[b] = jnp.where(same_head, jnp.broadcast_to(z, (C, C)), 0.0).astype(BF)
            kvb_s[b] = jnp.where(same_head, kv_s[b], 0.0).astype(BF)

    def reset_state():
        kv_s[...] = jnp.zeros(kv_s.shape, F32)
        z_s[...] = jnp.zeros(z_s.shape, F32)

    class Pacer:
        def __init__(self, pace_ref, tasks, count):
            self.ref, self.count, self.heads = pace_ref, count, []
            self.background = Background(tasks, count - LAG - SLACK)
            for _ in range(LAG):
                self.load_head()

        def slot(self, row):
            return pl.ds(pl.multiple_of(zero_ref[0] + row, 8), 8)

        def load_head(self):
            if len(self.heads) < self.count:
                self.heads.append(self.ref[self.slot(len(self.heads) * 8), :])

        def product(self, index, left, right_ref):
            right = halves(jnp.concatenate([self.heads[index], right_ref[8:, :]], axis=0))
            out = jnp.dot(left, right, preferred_element_type=F32)
            if REV:
                self.ref[self.slot(PIN + 8), :] = out[REV - 8:REV]
            for value in self.background.advance():
                self.ref[self.slot(PIN), :] = value
            self.load_head()
            return out

    def projection_step(s, j):
        tasks = [(short_conv_task(s, j), SHORT_STEPS)]
        fillers = [None] * 21
        fillers[POS[0]] = functools.partial(kernel_spectra, s, j)
        if s + 1 < NS:
            tasks.append((w_operand_task(s + 1, j), W_STEPS))
        if s == 0:
            tasks.append((left_operand_task(x_v, xs_s.at[j + 1], jnp.minimum(j + 1, NJ - 1)), LEFT_STEPS))
        if s >= 1:
            tasks.insert(0, (freq_conv_task(s - 1, j), FREQ_STEPS))
            fillers[POS[3]] = lambda: [normalise(s - 1, b, 2 * j + c) for b in range(2) for c in range(2)]
        if s >= 2:
            fillers[POS[1]] = functools.partial(conv_output, s - 2, j, 0)
            fillers[POS[2]] = functools.partial(conv_output, s - 2, j, 1)
        pacer = Pacer(pace[s % 2], tasks, 21)

        def emit(t, h, b, val):
            rows = aligned((j + NJ * h) * C, C)
            if t == 0:
                pq_s[s % 2, b, rows, :] = _phi(val)
            elif t == 1:
                pk = _phi(val)
                z_s[b] += jnp.sum(pk.reshape(C // 8, 8, C), axis=0)
                pkt_s[b, :, h * C:(h + 1) * C] = pk.T.astype(BF)
            else:
                vv_s[b, h * C:(h + 1) * C, :] = val.astype(BF)

        done = []
        for t in T_ORDER:
            def product(p, t=t):
                done.append(p)
                left = jnp.concatenate([halves(xs_s[j + zero_ref[1 + t], p, kt]) for kt in range(4)], axis=1)
                return pacer.product(len(done) - 1, left, ws[s % 2].at[t, p])
            _strassen(product, functools.partial(emit, t), fillers)
        input_spectra(s, j)
        if s >= 1:
            for b in range(2):
                fold_wo(s - 1, b, j)
        for b in range(2):
            kv_s[b] += jnp.dot(pkt_s[b], vv_s[b], preferred_element_type=F32)

    def super_step(s):
        if s >= 1:
            wait(inputs_of(s))
            start(inputs_of(s + 1))
        reset_state()
        publish_heads(pace[s % 2], ws[s % 2], T_ORDER)

        def body(j, carry):
            if s == 0:
                @pl.when((j + 1 < NJ) & (j % 2 == 1))
                def _():
                    wait(first_group((j + 1) // 2))

                @pl.when(j == START1)
                def _():
                    start(inputs_of(1))
            projection_step(s, j)
            return carry

        lax.fori_loop(0, NJ, body, 0, unroll=UN if s else 1)
        finish_state()
        if s >= 2:
            start(ob_copies(s - 2))

    def output_step(j, carry):
        fillers = [None] * 28
        for b in range(2):
            fillers[POS2[b]] = functools.partial(conv_output, NS - 2, j, b)
        fillers[POS2[2]] = functools.partial(normalise_pair, jnp.minimum(j + 2, NJ - 1))
        tasks = [(freq_conv_task(NS - 1, j), FREQ_STEPS),
                 (left_operand_task(op_s, os_s.at[(j + 1) % 2], jnp.minimum(j + 1, NJ - 1)), LEFT_STEPS)]
        pacer = Pacer(pace[NS % 2], tasks, 28)

        def emit(n, h, half, val):
            oa_v[j, h, :, (4 * half + n) * C:(4 * half + n + 1) * C] = val.astype(BF)

        done = []
        for n in range(4):
            def product(p, n=n):
                done.append(p)
                left = jnp.concatenate([halves(os_s[j % 2, p + zero_ref[n], kt]) for kt in range(4)], axis=1)
                return pacer.product(len(done) - 1, left, ms_s.at[n, p])
            _strassen(product, functools.partial(emit, n), fillers)
        start(oa_copies(j))
        return carry

    def normalise_pair(j):
        for b in range(2):
            for h in range(2):
                normalise(NS - 1, b, j + NJ * h)

    for t in T_ORDER:
        start(w_copies(0, 0, 1, (t,)))
    for g in range(NG):
        start(first_group(g))

    sh = shift_ref[...].astype(F32)
    dd = d_ref[...].astype(F32).reshape(1, D)
    for i in range(NB):
        par_s[i, 0:4, :] = sh[:, i * C:(i + 1) * C]
        par_s[i, 4:5, :] = dd[:, i * C:(i + 1) * C]
    kf_s[:, 0:8, :] = jnp.zeros((2, 8, C), F32)

    for t in T_ORDER:
        wait(w_copies(0, 0, 1, (t,)))

        def first_operands(j, carry, t=t):
            for _ in w_operand_task(0, j, (t,)):
                pass
            return carry

        lax.fori_loop(0, NJ, first_operands, 0, unroll=NJ)
    wait(first_group(0))
    run(left_operand_task(x_v, xs_s.at[0], 0))

    for s in range(NS):
        super_step(s)

    wait(inputs_of(NS))
    start(q_copies(NS - 1))
    normalise_pair(0)
    normalise_pair(1)
    run(left_operand_task(op_s, os_s.at[0], 0))
    for n in range(4):
        for b in range(2):
            fold_wo(NS - 1, b, n)
            fold_wo(NS - 1, b, 4 + n)
        m_operands(n)
    publish_heads(pace[NS % 2], ms_s, range(4))
    lax.fori_loop(0, NJ, output_step, 0, unroll=UN)
    start(ob_copies(NS - 2))
    wait(q_copies(NS - 1))
    for g in range(NG):
        for j in (2 * g, 2 * g + 1):
            for b in range(2):
                conv_output(NS - 1, j, b)
        start(ob_copies(NS - 1, g, NG))
    for s in range(NS - 1):
        wait(ob_copies(s))
    for j in range(NJ):
        wait(oa_copies(j))
    for g in range(NG):
        wait(ob_copies(NS - 1, g, NG))


def make(GS=64, GF=(8, 11, 14, 16), LAG=3, REV=8, SLACK=2, POS2=(10, 20, 27), GO=64, START1=3, UN=1, POS=(14, 3, 10, 17), flags=None):
    def fn(A_x, A_wqkv, A_wo, B_q, B_k, B_v, B_shift_k, B_ssm_k, B_ssm_D):
        hbm = pl.BlockSpec(memory_space=pl.ANY)
        vmem = pl.BlockSpec(memory_space=pltpu.VMEM)
        out = pl.pallas_call(
            functools.partial(_kernel, SLACK=SLACK, POS=POS, GO=GO, START1=START1, UN=UN, GS=GS, GF=GF, LAG=LAG, REV=REV, POS2=POS2),
            out_shape=jax.ShapeDtypeStruct((S, 2 * D), BF),
            in_specs=[pl.BlockSpec(memory_space=pltpu.SMEM)] + [hbm] * 7 + [vmem] * 4,
            out_specs=hbm,
            scratch_shapes=[
                pltpu.VMEM((PACE_ROWS, C), F32),
                pltpu.VMEM((PACE_ROWS, C), F32),
                pltpu.VMEM((NJ + 1, 7, 4, H, C), F32),
                pltpu.VMEM((3, 7, 4 * H, C), F32),
                pltpu.VMEM((3, 7, 4 * H, C), F32),
                pltpu.VMEM((2, NC, C, C), F32),
                pltpu.VMEM((2, NC, C, C), F32),
                pltpu.VMEM((2, S + 8, C), F32),
                pltpu.VMEM((4, H, C), F32),
                pltpu.VMEM((2, 6, NC, 8, C), F32),
                pltpu.VMEM((4, 7, 4 * H, C), F32),
                pltpu.VMEM((2, 7, 4, H, C), F32),
                pltpu.VMEM((NB, S, C), BF),
                pltpu.VMEM((NB, 3, D, C), BF),
                pltpu.VMEM((NS, 2 * C, D), BF),
                pltpu.VMEM((NB, S, C), BF),
                pltpu.VMEM((NB, S, C), BF),
                pltpu.VMEM((NB, S, C), BF),
                pltpu.VMEM((NB, C, S), BF),
                pltpu.VMEM((NB, S, C), BF),
                pltpu.VMEM((NJ, 2, C, D), BF),
                pltpu.VMEM((2, 2, S, C), F32),
                pltpu.VMEM((2, C, 2 * C), BF),
                pltpu.VMEM((2, 2 * C, C), BF),
                pltpu.VMEM((2, C, C), F32),
                pltpu.VMEM((2, 8, C), F32),
                pltpu.VMEM((2, C, C), BF),
                pltpu.VMEM((2, C, C), BF),
                pltpu.VMEM((NB, S, C), BF),
                pltpu.VMEM((NB, D, C), BF),
                pltpu.VMEM((NB, 8, C), F32),
                pltpu.SemaphoreType.DMA((NG,)),
                pltpu.SemaphoreType.DMA((NS, NG)),
                pltpu.SemaphoreType.DMA((NS, NG)),
                pltpu.SemaphoreType.DMA((2, NS)),
                pltpu.SemaphoreType.DMA((3, NB)),
            ],
            compiler_params=pltpu.CompilerParams(vmem_limit_bytes=120 * 2**20, flags=flags),
        )(
            jnp.asarray(np.zeros((4,), np.int32)),
            A_x.reshape(S, D), A_wqkv, A_wo,
            B_q.reshape(S, D), B_k.reshape(S, D), B_v.reshape(S, D),
            B_ssm_k, B_shift_k.T, B_ssm_D,
            jnp.asarray(_FWD.astype(BF)), jnp.asarray(_INV.astype(BF)),
        )
        return out.reshape(1, S, 2 * D)
    return jax.jit(fn)


_fn = make(GS=32)


@jax.jit
def pallas_concat_heads__linear_attn_block__ssm_conv_h3__prompt_kernel(
    A_x: jax.Array,
    A_wqkv: jax.Array,
    A_wo: jax.Array,
    B_q: jax.Array,
    B_k: jax.Array,
    B_v: jax.Array,
    B_shift_k: jax.Array,
    B_ssm_k: jax.Array,
    B_ssm_D: jax.Array,
):
    return _fn(A_x, A_wqkv, A_wo, B_q, B_k, B_v, B_shift_k, B_ssm_k, B_ssm_D)
```

```python
import functools

import jax
import jax.numpy as jnp
import numpy as np
from jax import lax
import jax.experimental.pallas as pl
import jax.experimental.pallas.tpu as pltpu

BF = jnp.bfloat16
F32 = jnp.float32
S = 2048
D = 1024
C = 128
H = C // 2
NC = S // C
NB = D // C
NS = NB // 2
NJ = NC // 2
DH = 32

PIN = 28 * 8
UH = PIN + 16
KH = UH + 2 * NC * 2 * C
PACE_ROWS = KH + 2 * NC * 2 * C

P_ORDER = (0, 5, 6, 1, 3, 4, 2)
NT = (((1,), (1,)), ((), ()))


def _dft_matrix():
    n = np.arange(C, dtype=np.float64)[None, :]
    m = np.arange(C, dtype=np.float64)[:, None]
    theta = 2.0 * np.pi * (m + 0.25) / C
    return np.concatenate([np.cos(theta * n), -np.sin(theta * n)], axis=0)


def _paired(n):
    pos = np.arange(n)
    return pos // 16 * 16 + pos % 2 * 8 + pos % 16 // 2


_FWD = np.stack([_dft_matrix(), _dft_matrix()[:, _paired(C)]]).astype(np.float32)
_INV = (_dft_matrix().T / C)[:, _paired(2 * C)].astype(np.float32)


def _phi(t):
    return jnp.where(t > 0, t + 1.0, jnp.exp(t)) + 1e-6


def _tree_sum(terms):
    while len(terms) > 1:
        terms = [terms[e] + terms[e + 1] if e + 1 < len(terms) else terms[e]
                 for e in range(0, len(terms), 2)]
    return terms[0]


def _pack_rows(even, odd):
    return pltpu.bitcast(pltpu.pack_elementwise([even, odd], packed_dtype=BF), F32)


class _Tile:
    def __init__(self, tile):
        bits = pltpu.bitcast(tile, jnp.uint32)
        self.words = pltpu.bitcast(bits, F32)
        self.even = pltpu.bitcast(bits << 16, F32)
        self.odd = pltpu.bitcast(bits & np.uint32(0xFFFF0000), F32)

    def __add__(self, other):
        return _pack_rows(self.even + other.even, self.odd + other.odd)

    def __sub__(self, other):
        return _pack_rows(self.even - other.even, self.odd - other.odd)


def _left_operands(*tiles):
    a11, a12, a21, a22 = (_Tile(t) for t in tiles)
    return [a11 + a22, a21 + a22, a11.words, a22.words, a11 + a12, a21 - a11, a12 - a22]


def _right_operands(*tiles):
    b11, b12, b21, b22 = (_Tile(t) for t in tiles)
    return [b11 + b22, b11.words, b12 - b22, b21 - b11, b22.words, b11 + b12, b21 + b22]


def _strassen(product, emit, fillers):
    def run(p):
        r = product(p)
        filler = fillers.pop(0)
        if filler is not None:
            filler()
        return r
    m = run(0)
    c11, c22 = m, m
    c22 = c22 + run(5)
    c11 = c11 + run(6)
    m = run(1)
    c21, c22 = m, c22 - m
    m = run(3)
    emit(1, 0, c21 + m)
    c11 = c11 + m
    m = run(4)
    emit(0, 0, c11 - m)
    c12 = m
    m = run(2)
    emit(0, 1, c12 + m)
    emit(1, 1, c22 + m)


class Background:
    def __init__(self, tasks, weights):
        self.tasks = [t for t, _ in tasks]
        self.total = [n for _, n in tasks]
        self.done = [0] * len(tasks)
        self.weights = weights
        self.slot = 0

    def advance(self):
        self.slot += 1
        share, whole = sum(self.weights[:self.slot]), sum(self.weights)
        for e, task in enumerate(self.tasks):
            while self.done[e] < -(-self.total[e] * share // whole):
                yield next(task)
                self.done[e] += 1


def _kernel(zero_ref, x_hbm, w_hbm, wo_hbm, q_hbm, k_hbm, v_hbm, sk_hbm, shift_ref, d_ref, f_ref, fi_ref,
            o_hbm,
            pace0, pace1, xs_s, ws0, ws1, yh0, yh1, kf_s, us_s, tm_s, ms_s, os_s, x_v, w_v, wo_v, q_v, k_v, v_v, sk_v, ob_v, oa_v,
            pq_s, pkt_s, vv_s, kv_s, z_s, kvb_s, zt_s, op_s, m_s, par_s,
            sem_x, sem_w, sem_in, sem_o, sem_b, *, T_ORDER, WT, WT2, FIRST, AHEAD, POS, GS, GF, GO, LAG, REV, POS2, UN):

    def aligned(start, size):
        return pl.ds(start if isinstance(start, int) else pl.multiple_of(start, size), size)

    pace, ws, yh = (pace0, pace1), (ws0, ws1), (yh0, yh1)

    def halves(tile):
        return pltpu.bitcast(tile, BF)

    def x_copies(j):
        return [pltpu.make_async_copy(x_hbm.at[aligned((j + NJ * h) * C, C), :],
                                      x_v.at[aligned((j + NJ * h) * C, C), :], sem_x.at[j]) for h in range(2)]

    def w_copies(s, rows, ts, sem):
        return [pltpu.make_async_copy(w_hbm.at[rows, pl.ds(t * D + s * 2 * C, 2 * C)], w_v.at[s, t, rows, :], sem)
                for t in ts]

    def step_inputs(s, j, action):
        sem = sem_in.at[s, j]
        span = aligned(j * 2 * C, 2 * C)
        cps = []
        if s < NS:
            cols = pl.ds(s * 2 * C, 2 * C)
            cps += [pltpu.make_async_copy(k_hbm.at[span, cols], k_v.at[s, span, :], sem),
                    pltpu.make_async_copy(v_hbm.at[span, cols], v_v.at[s, span, :], sem),
                    pltpu.make_async_copy(sk_hbm.at[cols, span], sk_v.at[s, :, span], sem)]
        if s + 1 < NS:
            for half in range(2):
                cps += w_copies(s + 1, aligned(half * (D // 2) + j * 64, 64), T_ORDER, sem)
        for e in ((s - 1,) if 1 <= s < NS - 1 else (s - 1, s) if s == NS - 1 else ()):
            cols = aligned(j * C, C)
            cps.append(pltpu.make_async_copy(wo_hbm.at[pl.ds(e * 2 * C, 2 * C), cols], wo_v.at[e, :, cols], sem))
        if s >= 2:
            cps.append(pltpu.make_async_copy(q_hbm.at[span, pl.ds((s - 2) * 2 * C, 2 * C)],
                                             q_v.at[s - 2, span, :], sem))
        action(cps)
        if s == 0:
            pl.when(j + 1 < NJ)(lambda: action(x_copies(jnp.minimum(j + 1, NJ - 1))))

    def all_inputs(s, action):
        for j in range(NJ):
            step_inputs(s, j, action)

    def ob_copy(s, j):
        rows = aligned(j * 2 * C, 2 * C)
        return pltpu.make_async_copy(ob_v.at[s, rows, :], o_hbm.at[rows, pl.ds(D + s * 2 * C, 2 * C)], sem_b.at[s, j])

    def oa_copies(j):
        return [pltpu.make_async_copy(oa_v.at[j, h], o_hbm.at[aligned((j + NJ * h) * C, C), pl.ds(0, D)],
                                      sem_o.at[h, j]) for h in range(2)]

    def start(cps):
        for cp in cps:
            cp.start()

    def wait(cps):
        for cp in cps:
            cp.wait()

    def short_conv_task(s, j):
        for b in range(2):
            i = 2 * s + b
            taps = [jnp.broadcast_to(par_s[i, e:e + 1, :], (8, C)) for e in range(4)]
            for c in range(2):
                r0 = (2 * j + c) * C
                kf_s[b, pl.ds(pl.multiple_of(r0 + 8, 8), C), :] = k_v[s, aligned(r0, C), b * C:(b + 1) * C].astype(F32)
                for r1 in range(0, C, GS):
                    vv = v_v[s, aligned(r0 + r1, GS), b * C:(b + 1) * C].astype(F32)
                    parts = []
                    for r in range(0, GS, 8):
                        ks = _tree_sum([kf_s[b, pl.ds(r0 + r1 + r + 8 - e, 8), :] * taps[e] for e in range(4)])
                        parts.append(ks * vv[r:r + 8])
                    us_s[2 * b + c, r1 // 2:(r1 + GS) // 2, :] = jnp.concatenate(
                        [_pack_rows(*parts[e:e + 2]) for e in range(0, len(parts), 2)], axis=0)
                    yield parts[-1]
    SHORT_STEPS = 4 * (C // GS)

    def freq_conv_task(s, j):
        src = pace[(s + 1) % 2]
        for b in range(2):
            skip = jnp.broadcast_to(par_s[2 * s + b, 4:5, :], (8, C))
            for t in range(3):
                for h in range(2):
                    def parts(base, a):
                        row = base + (b * NC + a) * 2 * C + j * 16 + 8 * h
                        return (lambda: src[aligned(row, 8), :]), (lambda: src[aligned(row + C, 8), :])

                    p, q, before = [], [], None
                    for a in range(NC):
                        if a == 0 or a in GF:
                            for e in range(a, min(g for g in GF if g > a)):
                                kr, ki = parts(KH, e)
                                ur, ui = parts(UH, e)
                                kr = kr() + skip if e == 0 else kr()
                                p.append(kr if t == 0 else ki() - kr if t == 1 else ki() + kr)
                                q.append(ur() + ui() if t == 0 else ur() if t == 1 else ui())
                        acc = _tree_sum([p[e] * q[a - e] for e in range(a + 1)])
                        if t == 0:
                            tm_s[b, h, a] = acc
                        elif t == 1:
                            acc = tm_s[b, h, a] + acc
                            tm_s[b, 2 + h, a] = acc
                        else:
                            re, im = tm_s[b, h, a] - acc, tm_s[b, 2 + h, a]
                            yr, yi = (re, im) if a == 0 else (re - before[1], im + before[0])
                            before, acc = (re, im), yr
                            if h == 0:
                                tm_s[b, 4, a] = yr
                                tm_s[b, 5, a] = yi
                            else:
                                yh[s % 2][b, a, aligned(j * 8, 8), :] = _pack_rows(tm_s[b, 4, a], yr)
                                yh[s % 2][b, a, aligned(H + j * 8, 8), :] = _pack_rows(tm_s[b, 5, a], yi)
                        if a + 1 in GF:
                            yield acc
    FREQ_STEPS = 2 * 3 * 2 * len(GF)

    def w_operand_task(s, j, ts=T_ORDER):
        for t in ts:
            top, bot = aligned(j * 64, 64), aligned(D // 2 + j * 64, 64)
            ops = _right_operands(w_v[s, t, top, :C], w_v[s, t, top, C:], w_v[s, t, bot, :C], w_v[s, t, bot, C:])
            for p in range(7):
                ws[s % 2][t, p, aligned(j * 32, 32), :] = ops[p]
            yield ops[6][:8]
    W_STEPS = 3

    def publish_heads(dst, src, order):
        for e, t in enumerate(order):
            for g, p in enumerate(P_ORDER):
                dst[pl.ds((e * 7 + g) * 8, 8), :] = src[t, p, 0:8, :]

    def left_operand_task(src, dst, j):
        for kt in range(4):
            for r in range(0, C, GO):
                top, bot = aligned(j * C + r, GO), aligned((j + NJ) * C + r, GO)
                lo, hi = pl.ds(kt * C, C), pl.ds(D // 2 + kt * C, C)
                ops = _left_operands(src[top, lo], src[top, hi], src[bot, lo], src[bot, hi])
                for p in range(7):
                    dst[p, kt, r // 2:(r + GO) // 2, :] = ops[p]
                yield ops[6][:8]
    LEFT_STEPS = 4 * (C // GO)

    def run(task):
        for _ in task:
            pass

    def m_operands(n):
        for kt in range(4):
            top, bot = pl.ds(kt * C, C), pl.ds(D // 2 + kt * C, C)
            ops = _right_operands(m_s[n, top, :], m_s[4 + n, top, :], m_s[n, bot, :], m_s[4 + n, bot, :])
            for p in range(7):
                ms_s[n, p, pl.ds(kt * H, H), :] = ops[p]

    def store_spectra(s, j, base, spec):
        for b in range(2):
            for c in range(2):
                row = pl.multiple_of(base + (b * NC + 2 * j + c) * 2 * C, 8)
                pace[(s + 1) % 2][pl.ds(row, 2 * C), :] = spec[:, (2 * b + c) * C:(2 * b + c + 1) * C]

    def kernel_spectra(s, j):
        taps = jnp.concatenate([sk_v[s, b * C:(b + 1) * C, aligned((2 * j + c) * C, C)]
                                for b in range(2) for c in range(2)], axis=0)
        spec = lax.dot_general(f_ref[0], taps, NT, preferred_element_type=F32)
        store_spectra(s, j, KH, spec)

    def input_spectra(s, j):
        u = jnp.concatenate([halves(us_s[e]) for e in range(4)], axis=1)
        spec = jnp.dot(f_ref[1], u, preferred_element_type=F32)
        store_spectra(s, j, UH, spec)

    def conv_output(s, j, b):
        cols = slice(b * C, (b + 1) * C)
        spec = jnp.concatenate([pltpu.bitcast(yh[s % 2][b, 2 * j + c], BF) for c in range(2)], axis=1)
        y = jnp.dot(fi_ref[...], spec, preferred_element_type=F32)
        for c in range(2):
            rows = aligned((2 * j + c) * C, C)
            ob_v[s, rows, cols] = (y[:, c * C:(c + 1) * C] * q_v[s, rows, cols].astype(F32)).astype(BF)

    def normalise(s, b, a):
        rows = aligned(a * C, C)
        pq = pq_s[s % 2, b, rows, :]
        den = lax.dot_general(pq.astype(BF), zt_s[b], NT, preferred_element_type=F32) + 1e-6
        r = pl.reciprocal(den, approx=True)
        r = r * (2.0 - den * r)
        op_s[rows, (2 * s + b) * C:(2 * s + b + 1) * C] = (pq * r).astype(BF)

    def fold_wo(s, b, n):
        wo = wo_v[s, pl.ds(b * C, C), aligned(n * C, C)]
        m_s[n, aligned((2 * s + b) * C, C), :] = jnp.dot(kvb_s[b], wo, preferred_element_type=F32).astype(BF)

    def finish_state():
        same_head = (lax.broadcasted_iota(jnp.int32, (C, C), 0) // DH
                     == lax.broadcasted_iota(jnp.int32, (C, C), 1) // DH)
        for b in range(2):
            z = jnp.sum(z_s[b], axis=0, keepdims=True)
            zt_s[b] = jnp.where(same_head, jnp.broadcast_to(z, (C, C)), 0.0).astype(BF)
            kvb_s[b] = jnp.where(same_head, kv_s[b], 0.0).astype(BF)

    def reset_state():
        kv_s[...] = jnp.zeros(kv_s.shape, F32)
        z_s[...] = jnp.zeros(z_s.shape, F32)

    class Pacer:
        def __init__(self, pace_ref, tasks, weights):
            self.ref, self.count, self.heads = pace_ref, len(weights) - 1, []
            self.background = Background(tasks, weights)
            for _ in range(LAG - 1):
                self.load_head()
            self.run()

        def run(self):
            for value in self.background.advance():
                self.ref[self.slot(PIN), :] = value
            self.load_head()

        def slot(self, row):
            return pl.ds(pl.multiple_of(zero_ref[0] + row, 8), 8)

        def load_head(self):
            if len(self.heads) < self.count:
                self.heads.append(self.ref[self.slot(len(self.heads) * 8), :])

        def product(self, index, left, right_ref):
            right = halves(jnp.concatenate([self.heads[index], right_ref[8:, :]], axis=0))
            out = jnp.dot(left, right, preferred_element_type=F32)
            if REV:
                self.ref[self.slot(PIN + 8), :] = out[REV - 8:REV]
            self.run()
            return out

    def projection_step(s, j):
        tasks = [(short_conv_task(s, j), SHORT_STEPS)]
        fillers = [None] * 21
        fillers[POS[0]] = functools.partial(kernel_spectra, s, j)
        if s + 1 < NS:
            tasks.append((w_operand_task(s + 1, j), W_STEPS))
        if s == 0:
            tasks.append((left_operand_task(x_v, xs_s.at[j + 1], jnp.minimum(j + 1, NJ - 1)), LEFT_STEPS))
        if s >= 1:
            tasks.insert(0, (freq_conv_task(s - 1, j), FREQ_STEPS))
            fillers[POS[3]] = lambda: [normalise(s - 1, b, 2 * j + c) for b in range(2) for c in range(2)]
        if s >= 2:
            fillers[POS[1]] = functools.partial(conv_output, s - 2, j, 0)
            fillers[POS[2]] = functools.partial(conv_output, s - 2, j, 1)
        pacer = Pacer(pace[s % 2], tasks, WT)

        def emit(t, h, b, val):
            rows = aligned((j + NJ * h) * C, C)
            if t == 0:
                pq_s[s % 2, b, rows, :] = _phi(val)
            elif t == 1:
                pk = _phi(val)
                z_s[b] += jnp.sum(pk.reshape(C // 8, 8, C), axis=0)
                pkt_s[b, :, h * C:(h + 1) * C] = pk.T.astype(BF)
            else:
                vv_s[b, h * C:(h + 1) * C, :] = val.astype(BF)

        done = []
        for t in T_ORDER:
            def product(p, t=t):
                done.append(p)
                left = jnp.concatenate([halves(xs_s[j + zero_ref[1 + t], p, kt]) for kt in range(4)], axis=1)
                return pacer.product(len(done) - 1, left, ws[s % 2].at[t, p])
            _strassen(product, functools.partial(emit, t), fillers)
        input_spectra(s, j)
        if s >= 1:
            for b in range(2):
                fold_wo(s - 1, b, j)
        for b in range(2):
            kv_s[b] += jnp.dot(pkt_s[b], vv_s[b], preferred_element_type=F32)

    def super_step(s):
        if s >= 2:
            all_inputs(s, wait)
            all_inputs(s + 1, start)
        reset_state()
        publish_heads(pace[s % 2], ws[s % 2], T_ORDER)

        def body(j, carry):
            if s < 2:
                step_inputs(s, j, wait)
                pl.when(j + AHEAD < NJ)(lambda: step_inputs(s, jnp.minimum(j + AHEAD, NJ - 1), start))
                if s == 0:
                    pl.when(j + AHEAD >= NJ)(lambda: step_inputs(1, jnp.maximum(j + AHEAD - NJ, 0), start))
                else:
                    step_inputs(2, j, start)
            projection_step(s, j)
            if s >= 2:
                ob_copy(s - 2, j).start()
            return carry

        lax.fori_loop(0, NJ, body, 0, unroll=UN if s else 1)
        finish_state()

    def output_step(j, carry):
        fillers = [None] * 28
        for b in range(2):
            fillers[POS2[b]] = functools.partial(conv_output, NS - 2, j, b)
        fillers[POS2[2]] = functools.partial(normalise_pair, jnp.minimum(j + 2, NJ - 1))
        tasks = [(freq_conv_task(NS - 1, j), FREQ_STEPS),
                 (left_operand_task(op_s, os_s.at[(j + 1) % 2], jnp.minimum(j + 1, NJ - 1)), LEFT_STEPS)]
        pacer = Pacer(pace[NS % 2], tasks, WT2)

        def emit(n, h, half, val):
            oa_v[j, h, :, (4 * half + n) * C:(4 * half + n + 1) * C] = val.astype(BF)

        done = []
        for n in range(4):
            def product(p, n=n):
                done.append(p)
                left = jnp.concatenate([halves(os_s[j % 2, p + zero_ref[n], kt]) for kt in range(4)], axis=1)
                return pacer.product(len(done) - 1, left, ms_s.at[n, p])
            _strassen(product, functools.partial(emit, n), fillers)
        start(oa_copies(j) + [ob_copy(NS - 2, j)])
        return carry

    def normalise_pair(j):
        for b in range(2):
            for h in range(2):
                normalise(NS - 1, b, j + NJ * h)

    for t in T_ORDER:
        start(w_copies(0, pl.ds(0, D), (t,), sem_w.at[t]))
    start(x_copies(0))

    sh = shift_ref[...].astype(F32)
    dd = d_ref[...].astype(F32).reshape(1, D)
    for i in range(NB):
        par_s[i, 0:4, :] = sh[:, i * C:(i + 1) * C]
        par_s[i, 4:5, :] = dd[:, i * C:(i + 1) * C]
    kf_s[:, 0:8, :] = jnp.zeros((2, 8, C), F32)

    for t in T_ORDER:
        wait(w_copies(0, pl.ds(0, D), (t,), sem_w.at[t]))
        if t == T_ORDER[FIRST]:
            for j in range(AHEAD):
                step_inputs(0, j, start)

        def first_operands(j, carry, t=t):
            for _ in w_operand_task(0, j, (t,)):
                pass
            return carry

        lax.fori_loop(0, NJ, first_operands, 0, unroll=NJ)
    wait(x_copies(0))
    run(left_operand_task(x_v, xs_s.at[0], 0))

    for s in range(NS):
        super_step(s)

    normalise_pair(0)
    normalise_pair(1)
    run(left_operand_task(op_s, os_s.at[0], 0))
    for n in range(4):
        for b in range(2):
            fold_wo(NS - 1, b, n)
            fold_wo(NS - 1, b, 4 + n)
        m_operands(n)
    publish_heads(pace[NS % 2], ms_s, range(4))
    all_inputs(NS, wait)
    all_inputs(NS + 1, start)
    lax.fori_loop(0, NJ, output_step, 0, unroll=UN)
    all_inputs(NS + 1, wait)
    for j in range(NJ):
        for b in range(2):
            conv_output(NS - 1, j, b)
        ob_copy(NS - 1, j).start()
    for j in range(NJ):
        wait(oa_copies(j) + [ob_copy(s, j) for s in range(NS)])


WA = (2, 2, 2, 2, 2, 1, 1, 1, 2, 2, 2, 2, 1, 1, 1, 2, 2, 2, 2, 0, 0, 0)
WB = (1, 1, 2, 2, 2, 1, 1, 1, 2, 2, 2, 2, 1, 1, 1, 2, 2, 2, 2, 0, 0, 0)
WC = (1, 2, 3, 3, 3, 2, 2, 3, 3, 3, 3, 2, 2, 3, 3, 3, 3, 3, 2, 0, 0, 0)
WD = (1, 1, 2, 2, 2, 2, 1, 2, 2, 2, 2, 1, 2, 2, 2, 2, 2, 2, 1, 0, 0, 0)
WE = (0, 1, 2, 2, 2, 2, 2, 2, 2, 2, 1, 1, 2, 2, 2, 2, 2, 2, 2, 0, 0, 0)


def make(GS=64, GF=(6, 9, 11, 13, 15, 16), LAG=3, REV=8, T_ORDER=(1, 0, 2), WT=WE, WT2=(1,) * 26 + (0,) * 3, FIRST=0, AHEAD=2, POS2=(10, 20, 27), GO=32, UN=1, POS=(6, 12, 13, 17), flags=None):
    def fn(A_x, A_wqkv, A_wo, B_q, B_k, B_v, B_shift_k, B_ssm_k, B_ssm_D):
        hbm = pl.BlockSpec(memory_space=pl.ANY)
        vmem = pl.BlockSpec(memory_space=pltpu.VMEM)
        out = pl.pallas_call(
            functools.partial(_kernel, T_ORDER=T_ORDER, WT=WT, WT2=WT2, FIRST=FIRST, AHEAD=AHEAD, POS=POS, GO=GO, UN=UN, GS=GS, GF=GF, LAG=LAG, REV=REV, POS2=POS2),
            out_shape=jax.ShapeDtypeStruct((S, 2 * D), BF),
            in_specs=[pl.BlockSpec(memory_space=pltpu.SMEM)] + [hbm] * 7 + [vmem] * 4,
            out_specs=hbm,
            scratch_shapes=[
                pltpu.VMEM((PACE_ROWS, C), F32),
                pltpu.VMEM((PACE_ROWS, C), F32),
                pltpu.VMEM((NJ + 1, 7, 4, H, C), F32),
                pltpu.VMEM((3, 7, 4 * H, C), F32),
                pltpu.VMEM((3, 7, 4 * H, C), F32),
                pltpu.VMEM((2, NC, C, C), F32),
                pltpu.VMEM((2, NC, C, C), F32),
                pltpu.VMEM((2, S + 8, C), F32),
                pltpu.VMEM((4, H, C), F32),
                pltpu.VMEM((2, 6, NC, 8, C), F32),
                pltpu.VMEM((4, 7, 4 * H, C), F32),
                pltpu.VMEM((2, 7, 4, H, C), F32),
                pltpu.VMEM((S, D), BF),
                pltpu.VMEM((NS, 3, D, 2 * C), BF),
                pltpu.VMEM((NS, 2 * C, D), BF),
                pltpu.VMEM((NS, S, 2 * C), BF),
                pltpu.VMEM((NS, S, 2 * C), BF),
                pltpu.VMEM((NS, S, 2 * C), BF),
                pltpu.VMEM((NS, 2 * C, S), BF),
                pltpu.VMEM((NS, S, 2 * C), BF),
                pltpu.VMEM((NJ, 2, C, D), BF),
                pltpu.VMEM((2, 2, S, C), F32),
                pltpu.VMEM((2, C, 2 * C), BF),
                pltpu.VMEM((2, 2 * C, C), BF),
                pltpu.VMEM((2, C, C), F32),
                pltpu.VMEM((2, 8, C), F32),
                pltpu.VMEM((2, C, C), BF),
                pltpu.VMEM((2, C, C), BF),
                pltpu.VMEM((S, D), BF),
                pltpu.VMEM((NB, D, C), BF),
                pltpu.VMEM((NB, 8, C), F32),
                pltpu.SemaphoreType.DMA((NJ,)),
                pltpu.SemaphoreType.DMA((3,)),
                pltpu.SemaphoreType.DMA((NS + 2, NJ)),
                pltpu.SemaphoreType.DMA((2, NJ)),
                pltpu.SemaphoreType.DMA((NS, NJ)),
            ],
            compiler_params=pltpu.CompilerParams(vmem_limit_bytes=120 * 2**20, flags=flags),
        )(
            jnp.asarray(np.zeros((4,), np.int32)),
            A_x.reshape(S, D), A_wqkv, A_wo,
            B_q.reshape(S, D), B_k.reshape(S, D), B_v.reshape(S, D),
            B_ssm_k, B_shift_k.T, B_ssm_D,
            jnp.asarray(_FWD.astype(BF)), jnp.asarray(_INV.astype(BF)),
        )
        return out.reshape(1, S, 2 * D)
    return jax.jit(fn)


_fn = make()


@jax.jit
def pallas_concat_heads__linear_attn_block__ssm_conv_h3__prompt_kernel(
    A_x: jax.Array,
    A_wqkv: jax.Array,
    A_wo: jax.Array,
    B_q: jax.Array,
    B_k: jax.Array,
    B_v: jax.Array,
    B_shift_k: jax.Array,
    B_ssm_k: jax.Array,
    B_ssm_D: jax.Array,
):
    return _fn(A_x, A_wqkv, A_wo, B_q, B_k, B_v, B_shift_k, B_ssm_k, B_ssm_D)
```

```python
import functools

import jax
import jax.numpy as jnp
import numpy as np
from jax import lax
import jax.experimental.pallas as pl
import jax.experimental.pallas.tpu as pltpu

BF = jnp.bfloat16
F32 = jnp.float32
S = 2048
D = 1024
C = 128
H = C // 2
NC = S // C
NB = D // C
NS = NB // 2
NJ = NC // 2
DH = 32

HP = H + 8
SP = 2 * C + 8
PIN = 28 * 8
UH = PIN + 16
KH = UH + 2 * NC * SP + 16
PACE_ROWS = KH + 2 * NC * SP

P_ORDER = (0, 5, 6, 1, 3, 4, 2)
NT = (((1,), (1,)), ((), ()))


def _dft_matrix():
    n = np.arange(C, dtype=np.float64)[None, :]
    m = np.arange(C, dtype=np.float64)[:, None]
    theta = 2.0 * np.pi * (m + 0.25) / C
    return np.concatenate([np.cos(theta * n), -np.sin(theta * n)], axis=0)


def _paired(n):
    pos = np.arange(n)
    return pos // 16 * 16 + pos % 2 * 8 + pos % 16 // 2


_FWD = np.stack([_dft_matrix(), _dft_matrix()[:, _paired(C)]]).astype(np.float32)
_INV = (_dft_matrix().T / C)[:, _paired(2 * C)].astype(np.float32)


def _phi(t):
    return jnp.where(t > 0, t + 1.0, jnp.exp(t)) + 1e-6


def _tree_sum(terms):
    while len(terms) > 1:
        terms = [terms[e] + terms[e + 1] if e + 1 < len(terms) else terms[e]
                 for e in range(0, len(terms), 2)]
    return terms[0]


def _pack_rows(even, odd):
    return pltpu.bitcast(pltpu.pack_elementwise([even, odd], packed_dtype=BF), F32)


class _Tile:
    def __init__(self, tile):
        bits = pltpu.bitcast(tile, jnp.uint32)
        self.words = pltpu.bitcast(bits, F32)
        self.even = pltpu.bitcast(bits << 16, F32)
        self.odd = pltpu.bitcast(bits & np.uint32(0xFFFF0000), F32)

    def __add__(self, other):
        return _pack_rows(self.even + other.even, self.odd + other.odd)

    def __sub__(self, other):
        return _pack_rows(self.even - other.even, self.odd - other.odd)


def _left_operands(*tiles):
    a11, a12, a21, a22 = (_Tile(t) for t in tiles)
    return [a11 + a22, a21 + a22, a11.words, a22.words, a11 + a12, a21 - a11, a12 - a22]


def _right_operands(*tiles):
    b11, b12, b21, b22 = (_Tile(t) for t in tiles)
    return [b11 + b22, b11.words, b12 - b22, b21 - b11, b22.words, b11 + b12, b21 + b22]


def _strassen(product, emit, fillers):
    def run(p):
        r = product(p)
        filler = fillers.pop(0)
        if filler is not None:
            filler()
        return r
    m = run(0)
    c11, c22 = m, m
    c22 = c22 + run(5)
    c11 = c11 + run(6)
    m = run(1)
    c21, c22 = m, c22 - m
    m = run(3)
    emit(1, 0, c21 + m)
    c11 = c11 + m
    m = run(4)
    emit(0, 0, c11 - m)
    c12 = m
    m = run(2)
    emit(0, 1, c12 + m)
    emit(1, 1, c22 + m)


class Background:
    def __init__(self, tasks, weights):
        self.tasks = [t for t, _ in tasks]
        self.total = [n for _, n in tasks]
        self.done = [0] * len(tasks)
        self.weights = weights
        self.slot = 0

    def advance(self):
        self.slot += 1
        share, whole = sum(self.weights[:self.slot]), sum(self.weights)
        for e, task in enumerate(self.tasks):
            while self.done[e] < -(-self.total[e] * share // whole):
                yield next(task)
                self.done[e] += 1


def _kernel(zero_ref, x_hbm, w_hbm, wo_hbm, q_hbm, k_hbm, v_hbm, sk_hbm, shift_ref, d_ref, f_ref, fi_ref,
            o_hbm,
            pace0, pace1, xs_s, ws0, ws1, yh0, yh1, kf_s, us_s, tm_s, ms_s, os_s, x_v, w_v, wo_v, q_v, k_v, v_v, sk_v, ob_v, oa_v,
            pq_s, pkt_s, vv_s, kv_s, z_s, kvb_s, zt_s, op_s, m_s, par_s,
            sem_x, sem_w, sem_in, sem_o, sem_b, *, T_ORDER, WT, WT0, POS0, WT2, FIRST, AHEAD, POS, GS, GF, GO, LAG, REV, POS2, UN):

    def aligned(start, size):
        return pl.ds(start if isinstance(start, int) else pl.multiple_of(start, size), size)

    pace, ws, yh = (pace0, pace1), (ws0, ws1), (yh0, yh1)

    def halves(tile):
        return pltpu.bitcast(tile, BF)

    def x_copies(j):
        rows = aligned(j * C, C)
        return [pltpu.make_async_copy(x_hbm.at[:, rows, :], x_v.at[:, rows, :], sem_x.at[j])]

    def w_copies(s, rows, ts, sem):
        return [pltpu.make_async_copy(w_hbm.at[:, rows, pl.ds(t * D + s * 2 * C, 2 * C)],
                                      w_v.at[s, t, :, rows, :], sem) for t in ts]

    def step_inputs(s, j, action):
        sem = sem_in.at[s, j]
        span = aligned(j * 2 * C, 2 * C)
        cps = []
        if s < NS:
            cols = pl.ds(s * 2 * C, 2 * C)
            cps += [pltpu.make_async_copy(k_hbm.at[span, cols], k_v.at[s, span, :], sem),
                    pltpu.make_async_copy(v_hbm.at[span, cols], v_v.at[s, span, :], sem),
                    pltpu.make_async_copy(sk_hbm.at[cols, span], sk_v.at[s, :, span], sem)]
        if s + 1 < NS:
            cps += w_copies(s + 1, aligned(j * 64, 64), T_ORDER, sem)
        for e in ((s - 1,) if 1 <= s < NS - 1 else (s - 1, s) if s == NS - 1 else ()):
            cols = aligned(j * C, C)
            cps.append(pltpu.make_async_copy(wo_hbm.at[pl.ds(e * 2 * C, 2 * C), cols], wo_v.at[e, :, cols], sem))
        if s >= 2:
            cps.append(pltpu.make_async_copy(q_hbm.at[span, pl.ds((s - 2) * 2 * C, 2 * C)],
                                             q_v.at[s - 2, span, :], sem))
        action(cps)
        if s == 0:
            pl.when(j + 1 < NJ)(lambda: action(x_copies(jnp.minimum(j + 1, NJ - 1))))

    def all_inputs(s, action):
        for j in range(NJ):
            step_inputs(s, j, action)

    def ob_copy(s, j):
        rows = aligned(j * 2 * C, 2 * C)
        return pltpu.make_async_copy(ob_v.at[s, rows, :], o_hbm.at[rows, pl.ds(D + s * 2 * C, 2 * C)], sem_b.at[s, j])

    def oa_copies(j):
        return [pltpu.make_async_copy(oa_v.at[j, h], o_hbm.at[aligned((j + NJ * h) * C, C), pl.ds(0, D)],
                                      sem_o.at[h, j]) for h in range(2)]

    def start(cps):
        for cp in cps:
            cp.start()

    def wait(cps):
        for cp in cps:
            cp.wait()

    def short_conv_task(s, j):
        for b in range(2):
            i = 2 * s + b
            taps = [jnp.broadcast_to(par_s[i, e:e + 1, :], (8, C)) for e in range(4)]
            for c in range(2):
                r0 = (2 * j + c) * C
                kf_s[b, pl.ds(pl.multiple_of(r0 + 8, 8), C), :] = k_v[s, aligned(r0, C), b * C:(b + 1) * C].astype(F32)
                for r1 in range(0, C, GS):
                    vv = v_v[s, aligned(r0 + r1, GS), b * C:(b + 1) * C].astype(F32)
                    parts = []
                    for r in range(0, GS, 8):
                        ks = _tree_sum([kf_s[b, pl.ds(r0 + r1 + r + 8 - e, 8), :] * taps[e] for e in range(4)])
                        parts.append(ks * vv[r:r + 8])
                    us_s[2 * b + c, r1 // 2:(r1 + GS) // 2, :] = jnp.concatenate(
                        [_pack_rows(*parts[e:e + 2]) for e in range(0, len(parts), 2)], axis=0)
                    yield parts[-1]
    SHORT_STEPS = 4 * (C // GS)

    def freq_conv_task(s, j):
        src = pace[(s + 1) % 2]
        for b in range(2):
            skip = jnp.broadcast_to(par_s[2 * s + b, 4:5, :], (8, C))
            for t in range(3):
                for h in range(2):
                    def parts(base, a):
                        row = base + (b * NC + a) * SP + j * 16 + 8 * h
                        return (lambda: src[aligned(row, 8), :]), (lambda: src[aligned(row + C, 8), :])

                    p, q, before = [], [], None
                    for a in range(NC):
                        if a == 0 or a in GF:
                            for e in range(a, min(g for g in GF if g > a)):
                                kr, ki = parts(KH, e)
                                ur, ui = parts(UH, e)
                                kr = kr() + skip if e == 0 else kr()
                                p.append(kr if t == 0 else ki() - kr if t == 1 else ki() + kr)
                                q.append(ur() + ui() if t == 0 else ur() if t == 1 else ui())
                        acc = _tree_sum([p[e] * q[a - e] for e in range(a + 1)])
                        if t == 0:
                            tm_s[b, h, a] = acc
                        elif t == 1:
                            acc = tm_s[b, h, a] + acc
                            tm_s[b, 2 + h, a] = acc
                        else:
                            re, im = tm_s[b, h, a] - acc, tm_s[b, 2 + h, a]
                            yr, yi = (re, im) if a == 0 else (re - before[1], im + before[0])
                            before, acc = (re, im), yr
                            if h == 0:
                                tm_s[b, 4, a] = yr
                                tm_s[b, 5, a] = yi
                            else:
                                yh[s % 2][b, a, 0, aligned(j * 8, 8), :] = _pack_rows(tm_s[b, 4, a], yr)
                                yh[s % 2][b, a, 1, aligned(j * 8, 8), :] = _pack_rows(tm_s[b, 5, a], yi)
                        if a + 1 in GF:
                            yield acc
    FREQ_STEPS = 2 * 3 * 2 * len(GF)

    def w_operand_task(s, j, ts=T_ORDER):
        for t in ts:
            rows = aligned(j * 64, 64)
            ops = _right_operands(w_v[s, t, 0, rows, :C], w_v[s, t, 0, rows, C:],
                                  w_v[s, t, 1, rows, :C], w_v[s, t, 1, rows, C:])
            for p in range(7):
                ws[s % 2][t, p, j // 2, aligned(j % 2 * 32, 32), :] = ops[p]
            yield ops[6][:8]
    W_STEPS = 3

    def publish_heads(dst, src, order):
        for e, t in enumerate(order):
            for g, p in enumerate(P_ORDER):
                dst[pl.ds((e * 7 + g) * 8, 8), :] = src[t, p, 0, 0:8, :]

    def left_operand_task(src, dst, j):
        for kt in range(4):
            for r in range(0, C, GO):
                rows = aligned(j * C + r, GO)
                lo, hi = pl.ds(kt * C, C), pl.ds(D // 2 + kt * C, C)
                ops = _left_operands(src[0, rows, lo], src[0, rows, hi], src[1, rows, lo], src[1, rows, hi])
                for p in range(7):
                    dst[p, kt, r // 2:(r + GO) // 2, :] = ops[p]
                yield ops[6][:8]
    LEFT_STEPS = 4 * (C // GO)

    def run(task):
        for _ in task:
            pass

    def m_operands(n):
        for kt in range(4):
            top, bot = pl.ds(kt * C, C), pl.ds(D // 2 + kt * C, C)
            ops = _right_operands(m_s[n, top, :], m_s[4 + n, top, :], m_s[n, bot, :], m_s[4 + n, bot, :])
            for p in range(7):
                ms_s[n, p, kt, 0:H, :] = ops[p]

    def store_spectra(s, j, base, spec):
        for b in range(2):
            for c in range(2):
                row = pl.multiple_of(base + (b * NC + 2 * j + c) * SP, 8)
                pace[(s + 1) % 2][pl.ds(row, 2 * C), :] = spec[:, (2 * b + c) * C:(2 * b + c + 1) * C]

    def kernel_spectra(s, j):
        taps = jnp.concatenate([sk_v[s, b * C:(b + 1) * C, aligned((2 * j + c) * C, C)]
                                for b in range(2) for c in range(2)], axis=0)
        spec = lax.dot_general(f_ref[0], taps, NT, preferred_element_type=F32)
        store_spectra(s, j, KH, spec)

    def input_spectra(s, j):
        u = jnp.concatenate([halves(us_s[e, 0:H, :]) for e in range(4)], axis=1)
        spec = jnp.dot(f_ref[1], u, preferred_element_type=F32)
        store_spectra(s, j, UH, spec)

    def conv_output(s, j, b):
        cols = slice(b * C, (b + 1) * C)
        spec = jnp.concatenate([halves(jnp.concatenate([yh[s % 2][b, 2 * j + c, e, 0:H, :] for e in range(2)], axis=0))
                                for c in range(2)], axis=1)
        y = jnp.dot(fi_ref[...], spec, preferred_element_type=F32)
        for c in range(2):
            rows = aligned((2 * j + c) * C, C)
            ob_v[s, rows, cols] = (y[:, c * C:(c + 1) * C] * q_v[s, rows, cols].astype(F32)).astype(BF)

    def normalise(s, b, a):
        rows = aligned(a * C, C)
        pq = pq_s[s % 2, b, rows, :]
        den = lax.dot_general(pq.astype(BF), zt_s[b], NT, preferred_element_type=F32) + 1e-6
        r = pl.reciprocal(den, approx=True)
        r = r * (2.0 - den * r)
        op_s[a // NJ, aligned(a % NJ * C, C), (2 * s + b) * C:(2 * s + b + 1) * C] = (pq * r).astype(BF)

    def fold_wo(s, b, n):
        wo = wo_v[s, pl.ds(b * C, C), aligned(n * C, C)]
        m_s[n, aligned((2 * s + b) * C, C), :] = jnp.dot(kvb_s[b], wo, preferred_element_type=F32).astype(BF)

    def finish_state():
        same_head = (lax.broadcasted_iota(jnp.int32, (C, C), 0) // DH
                     == lax.broadcasted_iota(jnp.int32, (C, C), 1) // DH)
        for b in range(2):
            z = jnp.sum(z_s[b], axis=0, keepdims=True)
            zt_s[b] = jnp.where(same_head, jnp.broadcast_to(z, (C, C)), 0.0).astype(BF)
            kvb_s[b] = jnp.where(same_head, kv_s[b], 0.0).astype(BF)

    def reset_state():
        kv_s[...] = jnp.zeros(kv_s.shape, F32)
        z_s[...] = jnp.zeros(z_s.shape, F32)

    class Pacer:
        def __init__(self, pace_ref, tasks, weights):
            self.ref, self.count, self.heads = pace_ref, len(weights) - 1, []
            self.background = Background(tasks, weights)
            for _ in range(LAG - 1):
                self.load_head()
            self.run()

        def run(self):
            for value in self.background.advance():
                self.ref[self.slot(PIN), :] = value
            self.load_head()

        def slot(self, row):
            return pl.ds(pl.multiple_of(zero_ref[0] + row, 8), 8)

        def load_head(self):
            if len(self.heads) < self.count:
                self.heads.append(self.ref[self.slot(len(self.heads) * 8), :])

        def product(self, index, left, right_ref):
            right = halves(jnp.concatenate([self.heads[index], right_ref[0, 8:H, :]]
                                           + [right_ref[kt, 0:H, :] for kt in range(1, 4)], axis=0))
            out = jnp.dot(left, right, preferred_element_type=F32)
            if REV:
                self.ref[self.slot(PIN + 8), :] = out[REV - 8:REV]
            self.run()
            return out

    def projection_step(s, j):
        tasks = [(short_conv_task(s, j), SHORT_STEPS)]
        fillers = [None] * 21
        fillers[POS[0] if s else POS0] = functools.partial(kernel_spectra, s, j)
        if s + 1 < NS:
            tasks.append((w_operand_task(s + 1, j), W_STEPS))
        if s == 0:
            tasks.append((left_operand_task(x_v, xs_s.at[j + 1], jnp.minimum(j + 1, NJ - 1)), LEFT_STEPS))
        if s >= 1:
            tasks.insert(0, (freq_conv_task(s - 1, j), FREQ_STEPS))
            fillers[POS[3]] = lambda: [normalise(s - 1, b, 2 * j + c) for b in range(2) for c in range(2)]
        if s >= 2:
            fillers[POS[1]] = functools.partial(conv_output, s - 2, j, 0)
            fillers[POS[2]] = functools.partial(conv_output, s - 2, j, 1)
        pacer = Pacer(pace[s % 2], tasks, WT if s else WT0)

        def emit(t, h, b, val):
            rows = aligned((j + NJ * h) * C, C)
            if t == 0:
                pq_s[s % 2, b, rows, :] = _phi(val)
            elif t == 1:
                pk = _phi(val)
                z_s[b] += jnp.sum(pk.reshape(C // 8, 8, C), axis=0)
                pkt_s[b, :, h * C:(h + 1) * C] = pk.T.astype(BF)
            else:
                vv_s[b, h * C:(h + 1) * C, :] = val.astype(BF)

        done = []
        for t in T_ORDER:
            def product(p, t=t):
                done.append(p)
                left = jnp.concatenate([halves(xs_s[j + zero_ref[1 + t], p, kt, 0:H, :]) for kt in range(4)], axis=1)
                return pacer.product(len(done) - 1, left, ws[s % 2].at[t, p])
            _strassen(product, functools.partial(emit, t), fillers)
        input_spectra(s, j)
        if s >= 1:
            for b in range(2):
                fold_wo(s - 1, b, j)
        for b in range(2):
            kv_s[b] += jnp.dot(pkt_s[b], vv_s[b], preferred_element_type=F32)

    def super_step(s):
        if s >= 2:
            all_inputs(s, wait)
            all_inputs(s + 1, start)
        reset_state()
        publish_heads(pace[s % 2], ws[s % 2], T_ORDER)

        def body(j, carry):
            if s < 2:
                step_inputs(s, j, wait)
                pl.when(j + AHEAD < NJ)(lambda: step_inputs(s, jnp.minimum(j + AHEAD, NJ - 1), start))
                if s == 0:
                    pl.when(j + AHEAD >= NJ)(lambda: step_inputs(1, jnp.maximum(j + AHEAD - NJ, 0), start))
                else:
                    step_inputs(2, j, start)
            projection_step(s, j)
            if s >= 2:
                ob_copy(s - 2, j).start()
            return carry

        lax.fori_loop(0, NJ, body, 0, unroll=UN if s else 1)
        finish_state()

    def output_step(j, carry):
        fillers = [None] * 28
        for b in range(2):
            fillers[POS2[b]] = functools.partial(conv_output, NS - 2, j, b)
        fillers[POS2[2]] = functools.partial(normalise_pair, jnp.minimum(j + 2, NJ - 1))
        tasks = [(freq_conv_task(NS - 1, j), FREQ_STEPS),
                 (left_operand_task(op_s, os_s.at[(j + 1) % 2], jnp.minimum(j + 1, NJ - 1)), LEFT_STEPS)]
        pacer = Pacer(pace[NS % 2], tasks, WT2)

        def emit(n, h, half, val):
            oa_v[j, h, :, (4 * half + n) * C:(4 * half + n + 1) * C] = val.astype(BF)

        done = []
        for n in range(4):
            def product(p, n=n):
                done.append(p)
                left = jnp.concatenate([halves(os_s[j % 2, p + zero_ref[n], kt, 0:H, :]) for kt in range(4)], axis=1)
                return pacer.product(len(done) - 1, left, ms_s.at[n, p])
            _strassen(product, functools.partial(emit, n), fillers)
        start(oa_copies(j) + [ob_copy(NS - 2, j)])
        return carry

    def normalise_pair(j):
        for b in range(2):
            for h in range(2):
                normalise(NS - 1, b, j + NJ * h)

    for t in T_ORDER:
        start(w_copies(0, pl.ds(0, D // 2), (t,), sem_w.at[t]))
    start(x_copies(0))
    for j in range(AHEAD):
        if FIRST[j] < 0:
            step_inputs(0, j, start)

    sh = shift_ref[...].astype(F32)
    dd = d_ref[...].astype(F32).reshape(1, D)
    for i in range(NB):
        par_s[i, 0:4, :] = sh[:, i * C:(i + 1) * C]
        par_s[i, 4:5, :] = dd[:, i * C:(i + 1) * C]
    kf_s[:, 0:8, :] = jnp.zeros((2, 8, C), F32)

    for t in T_ORDER:
        wait(w_copies(0, pl.ds(0, D // 2), (t,), sem_w.at[t]))
        for j in range(AHEAD):
            if FIRST[j] >= 0 and t == T_ORDER[FIRST[j]]:
                step_inputs(0, j, start)

        def first_operands(j, carry, t=t):
            for _ in w_operand_task(0, j, (t,)):
                pass
            return carry

        lax.fori_loop(0, NJ, first_operands, 0, unroll=NJ)
    wait(x_copies(0))
    run(left_operand_task(x_v, xs_s.at[0], 0))

    for s in range(NS):
        super_step(s)

    normalise_pair(0)
    normalise_pair(1)
    run(left_operand_task(op_s, os_s.at[0], 0))
    for n in range(4):
        for b in range(2):
            fold_wo(NS - 1, b, n)
            fold_wo(NS - 1, b, 4 + n)
        m_operands(n)
    publish_heads(pace[NS % 2], ms_s, range(4))
    all_inputs(NS, wait)
    all_inputs(NS + 1, start)
    lax.fori_loop(0, NJ, output_step, 0, unroll=UN)
    all_inputs(NS + 1, wait)
    for j in range(NJ):
        for b in range(2):
            conv_output(NS - 1, j, b)
        ob_copy(NS - 1, j).start()
    for j in range(NJ):
        wait(oa_copies(j) + [ob_copy(s, j) for s in range(NS)])


WA = (2, 2, 2, 2, 2, 1, 1, 1, 2, 2, 2, 2, 1, 1, 1, 2, 2, 2, 2, 0, 0, 0)
WB = (1, 1, 2, 2, 2, 1, 1, 1, 2, 2, 2, 2, 1, 1, 1, 2, 2, 2, 2, 0, 0, 0)
WC = (1, 2, 3, 3, 3, 2, 2, 3, 3, 3, 3, 2, 2, 3, 3, 3, 3, 3, 2, 0, 0, 0)
WD = (1, 1, 2, 2, 2, 2, 1, 2, 2, 2, 2, 1, 2, 2, 2, 2, 2, 2, 1, 0, 0, 0)
WE = (0, 1, 2, 2, 2, 2, 2, 2, 2, 2, 1, 1, 2, 2, 2, 2, 2, 2, 2, 0, 0, 0)


def make(GS=64, GF=(6, 9, 11, 13, 15, 16), LAG=3, REV=8, T_ORDER=(1, 0, 2), WT=(0,1,2,2,2,2,2,2,2,2,2,2,1,1,2,2,2,2,2,0,0,0), WT0=(0,)+(1,)*16+(0,)*5, POS0=20, WT2=(1,) * 26 + (0,) * 3, FIRST=(0, 2), AHEAD=2, POS2=(10, 20, 27), GO=32, UN=1, POS=(6, 12, 13, 17), flags=None):
    def fn(A_x, A_wqkv, A_wo, B_q, B_k, B_v, B_shift_k, B_ssm_k, B_ssm_D):
        hbm = pl.BlockSpec(memory_space=pl.ANY)
        vmem = pl.BlockSpec(memory_space=pltpu.VMEM)
        out = pl.pallas_call(
            functools.partial(_kernel, T_ORDER=T_ORDER, WT=WT, WT0=WT0, POS0=POS0, WT2=WT2, FIRST=FIRST, AHEAD=AHEAD, POS=POS, GO=GO, UN=UN, GS=GS, GF=GF, LAG=LAG, REV=REV, POS2=POS2),
            out_shape=jax.ShapeDtypeStruct((S, 2 * D), BF),
            in_specs=[pl.BlockSpec(memory_space=pltpu.SMEM)] + [hbm] * 7 + [vmem] * 4,
            out_specs=hbm,
            scratch_shapes=[
                pltpu.VMEM((PACE_ROWS, C), F32),
                pltpu.VMEM((PACE_ROWS, C), F32),
                pltpu.VMEM((NJ + 1, 7, 4, HP, C), F32),
                pltpu.VMEM((3, 7, 4, HP, C), F32),
                pltpu.VMEM((3, 7, 4, HP, C), F32),
                pltpu.VMEM((2, NC, 2, HP, C), F32),
                pltpu.VMEM((2, NC, 2, HP, C), F32),
                pltpu.VMEM((2, S + 8, C), F32),
                pltpu.VMEM((4, HP, C), F32),
                pltpu.VMEM((2, 6, NC + 1, 8, C), F32),
                pltpu.VMEM((4, 7, 4, HP, C), F32),
                pltpu.VMEM((2, 7, 4, HP, C), F32),
                pltpu.VMEM((2, S // 2, D), BF),
                pltpu.VMEM((NS, 3, 2, D // 2, 2 * C), BF),
                pltpu.VMEM((NS, 2 * C, D), BF),
                pltpu.VMEM((NS, S, 2 * C), BF),
                pltpu.VMEM((NS, S, 2 * C), BF),
                pltpu.VMEM((NS, S, 2 * C), BF),
                pltpu.VMEM((NS, 2 * C, S), BF),
                pltpu.VMEM((NS, S, 2 * C), BF),
                pltpu.VMEM((NJ, 2, C, D), BF),
                pltpu.VMEM((2, 2, S, C), F32),
                pltpu.VMEM((2, C, 2 * C), BF),
                pltpu.VMEM((2, 2 * C, C), BF),
                pltpu.VMEM((2, C, C), F32),
                pltpu.VMEM((2, 8, C), F32),
                pltpu.VMEM((2, C, C), BF),
                pltpu.VMEM((2, C, C), BF),
                pltpu.VMEM((2, S // 2, D), BF),
                pltpu.VMEM((NB, D, C), BF),
                pltpu.VMEM((NB, 8, C), F32),
                pltpu.SemaphoreType.DMA((NJ,)),
                pltpu.SemaphoreType.DMA((3,)),
                pltpu.SemaphoreType.DMA((NS + 2, NJ)),
                pltpu.SemaphoreType.DMA((2, NJ)),
                pltpu.SemaphoreType.DMA((NS, NJ)),
            ],
            compiler_params=pltpu.CompilerParams(vmem_limit_bytes=120 * 2**20, flags=flags),
        )(
            jnp.asarray(np.zeros((4,), np.int32)),
            A_x.reshape(2, S // 2, D), A_wqkv.reshape(2, D // 2, 3 * D), A_wo,
            B_q.reshape(S, D), B_k.reshape(S, D), B_v.reshape(S, D),
            B_ssm_k, B_shift_k.T, B_ssm_D,
            jnp.asarray(_FWD.astype(BF)), jnp.asarray(_INV.astype(BF)),
        )
        return out.reshape(1, S, 2 * D)
    return jax.jit(fn)


_fn = make()


@jax.jit
def pallas_concat_heads__linear_attn_block__ssm_conv_h3__prompt_kernel(
    A_x: jax.Array,
    A_wqkv: jax.Array,
    A_wo: jax.Array,
    B_q: jax.Array,
    B_k: jax.Array,
    B_v: jax.Array,
    B_shift_k: jax.Array,
    B_ssm_k: jax.Array,
    B_ssm_D: jax.Array,
):
    return _fn(A_x, A_wqkv, A_wo, B_q, B_k, B_v, B_shift_k, B_ssm_k, B_ssm_D)
```

```python
import functools

import jax
import jax.numpy as jnp
import numpy as np
from jax import lax
import jax.experimental.pallas as pl
import jax.experimental.pallas.tpu as pltpu

BF = jnp.bfloat16
F32 = jnp.float32
S = 2048
D = 1024
C = 128
H = C // 2
NC = S // C
NB = D // C
NS = NB // 2
NJ = NC // 2
DH = 32

HP = H + 8
SP = 2 * C + 8
PIN = 28 * 8
UH = PIN + 16
KH = UH + 2 * NC * SP + 16
PACE_ROWS = KH + 2 * NC * SP

PAD = 16
AHEAD = 2
LAG = 3
GS, GO = 64, 32
GF = (6, 9, 11, 13, 15, 16)
T_ORDER = (1, 0, 2)
P_ORDER = (1, 3, 0, 5, 6, 4, 2)
NT = (((1,), (1,)), ((), ()))


def _dft_matrix():
    n = np.arange(C, dtype=np.float64)[None, :]
    m = np.arange(C, dtype=np.float64)[:, None]
    theta = 2.0 * np.pi * (m + 0.25) / C
    return np.concatenate([np.cos(theta * n), -np.sin(theta * n)], axis=0)


def _paired(n):
    pos = np.arange(n)
    return pos // 16 * 16 + pos % 2 * 8 + pos % 16 // 2


_FWD = np.stack([_dft_matrix(), _dft_matrix()[:, _paired(C)]]).astype(np.float32)
_INV = (_dft_matrix().T / C)[:, _paired(2 * C)].astype(np.float32)


def _phi(t):
    return jnp.where(t > 0, t + 1.0, jnp.exp(t)) + 1e-6


def _tree_sum(terms):
    while len(terms) > 1:
        terms = [terms[e] + terms[e + 1] if e + 1 < len(terms) else terms[e]
                 for e in range(0, len(terms), 2)]
    return terms[0]


def _pack_rows(even, odd):
    return pltpu.bitcast(pltpu.pack_elementwise([even, odd], packed_dtype=BF), F32)


class _Tile:
    def __init__(self, tile):
        bits = pltpu.bitcast(tile, jnp.uint32)
        self.words = pltpu.bitcast(bits, F32)
        self.even = pltpu.bitcast(bits << 16, F32)
        self.odd = pltpu.bitcast(bits & np.uint32(0xFFFF0000), F32)

    def __add__(self, other):
        return _pack_rows(self.even + other.even, self.odd + other.odd)

    def __sub__(self, other):
        return _pack_rows(self.even - other.even, self.odd - other.odd)


def _left_operands(*tiles):
    a11, a12, a21, a22 = (_Tile(t) for t in tiles)
    return [a11 + a22, a21 + a22, a11.words, a22.words, a11 + a12, a21 - a11, a12 - a22]


def _right_operands(*tiles):
    b11, b12, b21, b22 = (_Tile(t) for t in tiles)
    return [b11 + b22, b11.words, b12 - b22, b21 - b11, b22.words, b11 + b12, b21 + b22]


def _strassen(product, emit, fillers):
    def run(p):
        r = product(p)
        filler = fillers.pop(0)
        if filler is not None:
            filler()
        return r
    m2, m4 = run(1), run(3)
    emit(1, 0, m2 + m4)
    m1 = run(0)
    c11, c22 = m4 + m1, m1 - m2
    c22 = c22 + run(5)
    c11 = c11 + run(6)
    m5 = run(4)
    emit(0, 0, c11 - m5)
    m3 = run(2)
    emit(0, 1, m5 + m3)
    emit(1, 1, c22 + m3)


class Background:
    def __init__(self, tasks, weights):
        self.tasks = [t for t, _ in tasks]
        self.total = [n for _, n in tasks]
        self.done = [0] * len(tasks)
        self.weights = weights
        self.slot = 0

    def advance(self):
        self.slot += 1
        share, whole = sum(self.weights[:self.slot]), sum(self.weights)
        for e, task in enumerate(self.tasks):
            while self.done[e] < -(-self.total[e] * share // whole):
                yield next(task)
                self.done[e] += 1


def _kernel(zero_ref, x_hbm, w_hbm, wo_hbm, q_hbm, k_hbm, v_hbm, sk_hbm, shift_ref, d_ref, f_ref, fi_ref,
            o_hbm,
            pace0, pace1, xs_s, ws0, ws1, yh0, yh1, kf_s, us_s, tm_s, ms_s, os_s, x_v, w_v, wo_v, q_v, k_v, v_v, sk_v, ob_v, oa_v,
            pq_s, pkt_s, vv_s, kv_s, z_s, kvb_s, zt_s, op_s, m_s, par_s,
            sem_x, sem_w, sem_in, sem_o, sem_b, *, SHARES, AFTER):

    def aligned(start, size):
        return pl.ds(start if isinstance(start, int) else pl.multiple_of(start, size), size)

    pace, ws, yh = (pace0, pace1), (ws0, ws1), (yh0, yh1)

    def halves(tile):
        return pltpu.bitcast(tile, BF)

    def x_copies(j):
        rows = aligned(j * C, C)
        return [pltpu.make_async_copy(x_hbm.at[:, rows, :], x_v.at[:, rows, :], sem_x.at[j])]

    def w_copies(s, rows, ts, sem):
        return [pltpu.make_async_copy(w_hbm.at[:, rows, pl.ds(t * D + s * 2 * C, 2 * C)],
                                      w_v.at[s, t, :, rows, :], sem) for t in ts]

    def step_inputs(s, j, action):
        sem = sem_in.at[s, j]
        span = aligned(j * 2 * C, 2 * C)
        cps = []
        if s < NS:
            cols = pl.ds(s * 2 * C, 2 * C)
            cps += [pltpu.make_async_copy(k_hbm.at[span, cols], k_v.at[s, span, :], sem),
                    pltpu.make_async_copy(v_hbm.at[span, cols], v_v.at[s, span, :], sem),
                    pltpu.make_async_copy(sk_hbm.at[cols, span], sk_v.at[s, :, span], sem)]
        if s + 1 < NS:
            cps += w_copies(s + 1, aligned(j * 64, 64), T_ORDER, sem)
        for e in ((s - 1,) if 1 <= s < NS - 1 else (s - 1, s) if s == NS - 1 else ()):
            cols = aligned(j * C, C)
            cps.append(pltpu.make_async_copy(wo_hbm.at[pl.ds(e * 2 * C, 2 * C), cols], wo_v.at[e, :, cols], sem))
        if s >= 2:
            cps.append(pltpu.make_async_copy(q_hbm.at[span, pl.ds((s - 2) * 2 * C, 2 * C)],
                                             q_v.at[s - 2, span, :], sem))
        action(cps)
        if s == 0:
            pl.when(j + 1 < NJ)(lambda: action(x_copies(jnp.minimum(j + 1, NJ - 1))))

    def all_inputs(s, action):
        for j in range(NJ):
            step_inputs(s, j, action)

    def ob_copy(s, j):
        rows = aligned(j * 2 * C, 2 * C)
        return pltpu.make_async_copy(ob_v.at[s, rows, :], o_hbm.at[rows, pl.ds(D + s * 2 * C, 2 * C)], sem_b.at[s, j])

    def oa_copies(j):
        return [pltpu.make_async_copy(oa_v.at[j, h], o_hbm.at[aligned((j + NJ * h) * C, C), pl.ds(0, D)],
                                      sem_o.at[h, j]) for h in range(2)]

    def start(cps):
        for cp in cps:
            cp.start()

    def wait(cps):
        for cp in cps:
            cp.wait()

    def short_conv_task(s, j):
        for b in range(2):
            i = 2 * s + b
            taps = [jnp.broadcast_to(par_s[i, e:e + 1, :], (8, C)) for e in range(4)]
            for c in range(2):
                r0 = (2 * j + c) * C
                kf_s[b, pl.ds(pl.multiple_of(r0 + 8, 8), C), :] = k_v[s, aligned(r0, C), b * C:(b + 1) * C].astype(F32)
                for r1 in range(0, C, GS):
                    vv = v_v[s, aligned(r0 + r1, GS), b * C:(b + 1) * C].astype(F32)
                    parts = []
                    for r in range(0, GS, 8):
                        ks = _tree_sum([kf_s[b, pl.ds(r0 + r1 + r + 8 - e, 8), :] * taps[e] for e in range(4)])
                        parts.append(ks * vv[r:r + 8])
                    us_s[2 * b + c, r1 // 2:(r1 + GS) // 2, :] = jnp.concatenate(
                        [_pack_rows(*parts[e:e + 2]) for e in range(0, len(parts), 2)], axis=0)
                    yield parts[-1]
    SHORT_STEPS = 4 * (C // GS)

    def freq_conv_task(s, j):
        src = pace[(s + 1) % 2]
        for b in range(2):
            skip = jnp.broadcast_to(par_s[2 * s + b, 4:5, :], (8, C))
            for t in range(3):
                for h in range(2):
                    def parts(base, a):
                        row = base + (b * NC + a) * SP + j * 16 + 8 * h
                        return (lambda: src[aligned(row, 8), :]), (lambda: src[aligned(row + C, 8), :])

                    p, q, before = [], [], None
                    for a in range(NC):
                        if a == 0 or a in GF:
                            for e in range(a, min(g for g in GF if g > a)):
                                kr, ki = parts(KH, e)
                                ur, ui = parts(UH, e)
                                kr = kr() + skip if e == 0 else kr()
                                p.append(kr if t == 0 else ki() - kr if t == 1 else ki() + kr)
                                q.append(ur() + ui() if t == 0 else ur() if t == 1 else ui())
                        acc = _tree_sum([p[e] * q[a - e] for e in range(a + 1)])
                        if t == 0:
                            tm_s[b, h, a] = acc
                        elif t == 1:
                            acc = tm_s[b, h, a] + acc
                            tm_s[b, 2 + h, a] = acc
                        else:
                            re, im = tm_s[b, h, a] - acc, tm_s[b, 2 + h, a]
                            yr, yi = (re, im) if a == 0 else (re - before[1], im + before[0])
                            before, acc = (re, im), yr
                            if h == 0:
                                tm_s[b, 4, a] = yr
                                tm_s[b, 5, a] = yi
                            else:
                                yh[s % 2][b, a, 0, aligned(j * 8, 8), :] = _pack_rows(tm_s[b, 4, a], yr)
                                yh[s % 2][b, a, 1, aligned(j * 8, 8), :] = _pack_rows(tm_s[b, 5, a], yi)
                        if a + 1 in GF:
                            yield acc
    FREQ_STEPS = 2 * 3 * 2 * len(GF)

    def w_operand_task(s, j, ts=T_ORDER):
        for t in ts:
            rows = aligned(j * 64, 64)
            ops = _right_operands(w_v[s, t, 0, rows, :C], w_v[s, t, 0, rows, C:],
                                  w_v[s, t, 1, rows, :C], w_v[s, t, 1, rows, C:])
            for p in range(7):
                ws[s % 2][t, p, j // 2, aligned(j % 2 * 32, 32), :] = ops[p]
            yield ops[6][:8]
    W_STEPS = 3

    def publish_heads(dst, src, order):
        for e, t in enumerate(order):
            for g, p in enumerate(P_ORDER):
                dst[pl.ds((e * 7 + g) * 8, 8), :] = src[t, p, 0, 0:8, :]

    def left_operand_task(src, dst, j):
        for kt in range(4):
            for r in range(0, C, GO):
                rows = aligned(j * C + r, GO)
                lo, hi = pl.ds(kt * C, C), pl.ds(D // 2 + kt * C, C)
                ops = _left_operands(src[0, rows, lo], src[0, rows, hi], src[1, rows, lo], src[1, rows, hi])
                for p in range(7):
                    dst[p, kt, r // 2:(r + GO) // 2, :] = ops[p]
                yield ops[6][:8]
    LEFT_STEPS = 4 * (C // GO)

    def run(task):
        for _ in task:
            pass

    def m_operands(n):
        for kt in range(4):
            top, bot = pl.ds(kt * C, C), pl.ds(D // 2 + kt * C, C)
            ops = _right_operands(m_s[n, top, :], m_s[4 + n, top, :], m_s[n, bot, :], m_s[4 + n, bot, :])
            for p in range(7):
                ms_s[n, p, kt, 0:H, :] = ops[p]

    def store_spectra(s, j, base, spec):
        for b in range(2):
            for c in range(2):
                row = pl.multiple_of(base + (b * NC + 2 * j + c) * SP, 8)
                pace[(s + 1) % 2][pl.ds(row, 2 * C), :] = spec[:, (2 * b + c) * C:(2 * b + c + 1) * C]

    def kernel_spectra(s, j):
        taps = jnp.concatenate([sk_v[s, b * C:(b + 1) * C, aligned((2 * j + c) * C, C)]
                                for b in range(2) for c in range(2)], axis=0)
        spec = lax.dot_general(f_ref[0], taps, NT, preferred_element_type=F32)
        store_spectra(s, j, KH, spec)

    def input_spectra(s, j):
        u = jnp.concatenate([halves(us_s[e, 0:H, :]) for e in range(4)], axis=1)
        spec = jnp.dot(f_ref[1], u, preferred_element_type=F32)
        store_spectra(s, j, UH, spec)

    def conv_output(s, j, b):
        cols = slice(b * C, (b + 1) * C)
        spec = jnp.concatenate([halves(jnp.concatenate([yh[s % 2][b, 2 * j + c, e, 0:H, :] for e in range(2)], axis=0))
                                for c in range(2)], axis=1)
        y = jnp.dot(fi_ref[...], spec, preferred_element_type=F32)
        for c in range(2):
            rows = aligned((2 * j + c) * C, C)
            ob_v[s, rows, cols] = (y[:, c * C:(c + 1) * C] * q_v[s, rows, cols].astype(F32)).astype(BF)

    def normalise(s, b, a):
        rows = aligned(a * C, C)
        pq = pq_s[s % 2, b, rows, :]
        den = lax.dot_general(pq.astype(BF), zt_s[b], NT, preferred_element_type=F32) + 1e-6
        r = pl.reciprocal(den, approx=True)
        r = r * (2.0 - den * r)
        op_s[a // NJ, aligned(a % NJ * C, C), (2 * s + b) * C:(2 * s + b + 1) * C] = (pq * r).astype(BF)

    def fold_wo(s, b, n):
        wo = wo_v[s, pl.ds(b * C, C), aligned(n * C, C)]
        m_s[n, aligned((2 * s + b) * C, C), :] = jnp.dot(kvb_s[b], wo, preferred_element_type=F32).astype(BF)

    def finish_state():
        same_head = (lax.broadcasted_iota(jnp.int32, (C, C), 0) // DH
                     == lax.broadcasted_iota(jnp.int32, (C, C), 1) // DH)
        for b in range(2):
            z = jnp.sum(z_s[b], axis=0, keepdims=True)
            zt_s[b] = jnp.where(same_head, jnp.broadcast_to(z, (C, C)), 0.0).astype(BF)
            kvb_s[b] = jnp.where(same_head, kv_s[b], 0.0).astype(BF)

    def reset_state():
        kv_s[...] = jnp.zeros(kv_s.shape, F32)
        z_s[...] = jnp.zeros(z_s.shape, F32)

    class Pacer:
        def __init__(self, pace_ref, tasks, weights):
            self.ref, self.count, self.heads = pace_ref, len(weights) - 1, []
            self.background = Background(tasks, weights)
            for _ in range(LAG - 1):
                self.load_head()
            self.run()

        def run(self):
            for value in self.background.advance():
                self.ref[self.slot(PIN), :] = value
            self.load_head()

        def slot(self, row):
            return pl.ds(pl.multiple_of(zero_ref[0] + row, 8), 8)

        def load_head(self):
            if len(self.heads) < self.count:
                self.heads.append(self.ref[self.slot(len(self.heads) * 8), :])

        def product(self, index, left, right_ref):
            right = halves(jnp.concatenate([self.heads[index], right_ref[0, 8:H, :]]
                                           + [right_ref[kt, 0:H, :] for kt in range(1, 4)], axis=0))
            out = jnp.dot(left, right, preferred_element_type=F32)
            self.ref[self.slot(PIN + 8), :] = out[:8]
            self.run()
            return out

    def projection_step(s, j):
        tasks = [(short_conv_task(s, j), SHORT_STEPS)]
        fillers = [None] * 21
        fillers[AFTER[s][0]] = functools.partial(kernel_spectra, s, j)
        if s + 1 < NS:
            tasks.append((w_operand_task(s + 1, j), W_STEPS))
        if s == 0:
            tasks.append((left_operand_task(x_v, xs_s.at[j + 1], jnp.minimum(j + 1, NJ - 1)), LEFT_STEPS))
        if s >= 1:
            tasks.insert(0, (freq_conv_task(s - 1, j), FREQ_STEPS))
            fillers[AFTER[s][1]] = lambda: [normalise(s - 1, b, 2 * j + c) for b in range(2) for c in range(2)]
        if s >= 2:
            fillers[AFTER[s][2]] = functools.partial(conv_output, s - 2, j, 0)
            fillers[AFTER[s][3]] = functools.partial(conv_output, s - 2, j, 1)
        pacer = Pacer(pace[s % 2], tasks, SHARES[s])

        def emit(t, h, b, val):
            rows = aligned((j + NJ * h) * C, C)
            if t == 0:
                pq_s[s % 2, b, rows, :] = _phi(val)
            elif t == 1:
                pk = _phi(val)
                z_s[b] += jnp.sum(pk.reshape(C // 8, 8, C), axis=0)
                pkt_s[b, :, h * C:(h + 1) * C] = pk.T.astype(BF)
            else:
                vv_s[b, h * C:(h + 1) * C, :] = val.astype(BF)

        done = []
        for t in T_ORDER:
            def product(p, t=t):
                done.append(p)
                left = jnp.concatenate([halves(xs_s[j + zero_ref[1 + t], p, kt, 0:H, :]) for kt in range(4)], axis=1)
                return pacer.product(len(done) - 1, left, ws[s % 2].at[t, p])
            _strassen(product, functools.partial(emit, t), fillers)
        input_spectra(s, j)
        if s >= 1:
            for b in range(2):
                fold_wo(s - 1, b, j)
        for b in range(2):
            kv_s[b] += jnp.dot(pkt_s[b], vv_s[b], preferred_element_type=F32)

    def super_step(s):
        if s >= 2:
            all_inputs(s, wait)
            all_inputs(s + 1, start)
        reset_state()
        publish_heads(pace[s % 2], ws[s % 2], T_ORDER)

        def body(j, carry):
            if s < 2:
                step_inputs(s, j, wait)
                pl.when(j + AHEAD < NJ)(lambda: step_inputs(s, jnp.minimum(j + AHEAD, NJ - 1), start))
                if s == 0:
                    pl.when(j + AHEAD >= NJ)(lambda: step_inputs(1, jnp.maximum(j + AHEAD - NJ, 0), start))
                else:
                    step_inputs(2, j, start)
            projection_step(s, j)
            if s >= 2:
                ob_copy(s - 2, j).start()
            return carry

        lax.fori_loop(0, NJ, body, 0)
        finish_state()

    def output_step(j, carry):
        fillers = [None] * 28
        for b in range(2):
            fillers[AFTER[NS][b]] = functools.partial(conv_output, NS - 2, j, b)
        fillers[AFTER[NS][2]] = functools.partial(normalise_pair, jnp.minimum(j + 2, NJ - 1))
        tasks = [(freq_conv_task(NS - 1, j), FREQ_STEPS),
                 (left_operand_task(op_s, os_s.at[(j + 1) % 2], jnp.minimum(j + 1, NJ - 1)), LEFT_STEPS)]
        pacer = Pacer(pace[NS % 2], tasks, SHARES[NS])

        def emit(n, h, half, val):
            oa_v[j, h, :, (4 * half + n) * C:(4 * half + n + 1) * C] = val.astype(BF)

        done = []
        for n in range(4):
            def product(p, n=n):
                done.append(p)
                left = jnp.concatenate([halves(os_s[j % 2, p + zero_ref[n], kt, 0:H, :]) for kt in range(4)], axis=1)
                return pacer.product(len(done) - 1, left, ms_s.at[n, p])
            _strassen(product, functools.partial(emit, n), fillers)
        start(oa_copies(j) + [ob_copy(NS - 2, j)])
        return carry

    def normalise_pair(j):
        for b in range(2):
            for h in range(2):
                normalise(NS - 1, b, j + NJ * h)

    for t in T_ORDER:
        start(w_copies(0, pl.ds(0, D // 2), (t,), sem_w.at[t]))
    start(x_copies(0))

    sh = shift_ref[...].astype(F32)
    dd = d_ref[...].astype(F32).reshape(1, D)
    for i in range(NB):
        par_s[i, 0:4, :] = sh[:, i * C:(i + 1) * C]
        par_s[i, 4:5, :] = dd[:, i * C:(i + 1) * C]
    kf_s[:, 0:8, :] = jnp.zeros((2, 8, C), F32)

    for t in T_ORDER:
        wait(w_copies(0, pl.ds(0, D // 2), (t,), sem_w.at[t]))
        if t != T_ORDER[1]:
            step_inputs(0, 0 if t == T_ORDER[0] else 1, start)

        def first_operands(j, carry, t=t):
            for _ in w_operand_task(0, j, (t,)):
                pass
            return carry

        lax.fori_loop(0, NJ, first_operands, 0, unroll=NJ)
    wait(x_copies(0))
    run(left_operand_task(x_v, xs_s.at[0], 0))

    for s in range(NS):
        super_step(s)

    normalise_pair(0)
    normalise_pair(1)
    run(left_operand_task(op_s, os_s.at[0], 0))
    for n in range(4):
        for b in range(2):
            fold_wo(NS - 1, b, n)
            fold_wo(NS - 1, b, 4 + n)
        m_operands(n)
    publish_heads(pace[NS % 2], ms_s, range(4))
    all_inputs(NS, wait)
    all_inputs(NS + 1, start)
    lax.fori_loop(0, NJ, output_step, 0)
    all_inputs(NS + 1, wait)
    for j in range(NJ):
        for b in range(2):
            conv_output(NS - 1, j, b)
        ob_copy(NS - 1, j).start()
    for j in range(NJ):
        wait(oa_copies(j) + [ob_copy(s, j) for s in range(NS)])


_SHARES = (
    (0,) + (1,) * 16 + (0,) * 5,
    (1, 1, 2, 2, 2, 2, 1, 1, 2, 2, 2, 2, 2, 1, 1, 2, 2, 2, 2, 0, 0, 0),
    (1, 1, 2, 2, 2, 1, 1, 1, 2, 2, 2, 2, 1, 1, 1, 2, 2, 2, 2, 0, 0, 0),
    (1, 1, 2, 2, 2, 1, 1, 1, 2, 2, 2, 2, 1, 1, 1, 2, 2, 2, 2, 0, 0, 0),
    (1,) * 26 + (0,) * 3,
)
_AFTER = ((20,), (6, 17), (6, 17, 12, 13), (13, 16, 1, 6), (10, 20, 27))


def make(SHARES=_SHARES, AFTER=_AFTER):
    def fn(A_x, A_wqkv, A_wo, B_q, B_k, B_v, B_shift_k, B_ssm_k, B_ssm_D):
        hbm = pl.BlockSpec(memory_space=pl.ANY)
        vmem = pl.BlockSpec(memory_space=pltpu.VMEM)
        out = pl.pallas_call(
            functools.partial(_kernel, SHARES=SHARES, AFTER=AFTER),
            out_shape=jax.ShapeDtypeStruct((S, 2 * D), BF),
            in_specs=[pl.BlockSpec(memory_space=pltpu.SMEM)] + [hbm] * 7 + [vmem] * 4,
            out_specs=hbm,
            scratch_shapes=[
                pltpu.VMEM((PACE_ROWS, C), F32),
                pltpu.VMEM((PACE_ROWS, C), F32),
                pltpu.VMEM((NJ + 1, 7, 4, HP, C), F32),
                pltpu.VMEM((3, 7, 4, HP, C), F32),
                pltpu.VMEM((3, 7, 4, HP, C), F32),
                pltpu.VMEM((2, NC, 2, HP, C), F32),
                pltpu.VMEM((2, NC, 2, HP, C), F32),
                pltpu.VMEM((2, S + 16, C), F32),
                pltpu.VMEM((4, HP, C), F32),
                pltpu.VMEM((2, 6, NC + 1, 8, C), F32),
                pltpu.VMEM((4, 7, 4, HP, C), F32),
                pltpu.VMEM((2, 7, 4, HP, C), F32),
                pltpu.VMEM((2, S // 2 + PAD, D), BF),
                pltpu.VMEM((NS, 3, 2, D // 2 + PAD, 2 * C), BF),
                pltpu.VMEM((NS, 2 * C, D), BF),
                pltpu.VMEM((NS, S, 2 * C), BF),
                pltpu.VMEM((NS, S, 2 * C), BF),
                pltpu.VMEM((NS, S, 2 * C), BF),
                pltpu.VMEM((NS, 2 * C, S), BF),
                pltpu.VMEM((NS, S, 2 * C), BF),
                pltpu.VMEM((NJ, 2, C, D), BF),
                pltpu.VMEM((2, 2, S, C), F32),
                pltpu.VMEM((2, C, 2 * C), BF),
                pltpu.VMEM((2, 2 * C, C), BF),
                pltpu.VMEM((2, C, C), F32),
                pltpu.VMEM((2, 8, C), F32),
                pltpu.VMEM((2, C, C), BF),
                pltpu.VMEM((2, C, C), BF),
                pltpu.VMEM((2, S // 2 + PAD, D), BF),
                pltpu.VMEM((NB, D, C), BF),
                pltpu.VMEM((NB, 8, C), F32),
                pltpu.SemaphoreType.DMA((NJ,)),
                pltpu.SemaphoreType.DMA((3,)),
                pltpu.SemaphoreType.DMA((NS + 2, NJ)),
                pltpu.SemaphoreType.DMA((2, NJ)),
                pltpu.SemaphoreType.DMA((NS, NJ)),
            ],
            compiler_params=pltpu.CompilerParams(
                vmem_limit_bytes=120 * 2**20, flags={'XLA_TPU_EVENLY_DISTRIBUTE_CRITICAL_NODES': True}),
        )(
            jnp.asarray(np.zeros((4,), np.int32)),
            A_x.reshape(2, S // 2, D), A_wqkv.reshape(2, D // 2, 3 * D), A_wo,
            B_q.reshape(S, D), B_k.reshape(S, D), B_v.reshape(S, D),
            B_ssm_k, B_shift_k.T, B_ssm_D,
            jnp.asarray(_FWD.astype(BF)), jnp.asarray(_INV.astype(BF)),
        )
        return out.reshape(1, S, 2 * D)
    return jax.jit(fn)


_fn = make()


@jax.jit
def pallas_concat_heads__linear_attn_block__ssm_conv_h3__prompt_kernel(
    A_x: jax.Array,
    A_wqkv: jax.Array,
    A_wo: jax.Array,
    B_q: jax.Array,
    B_k: jax.Array,
    B_v: jax.Array,
    B_shift_k: jax.Array,
    B_ssm_k: jax.Array,
    B_ssm_D: jax.Array,
):
    return _fn(A_x, A_wqkv, A_wo, B_q, B_k, B_v, B_shift_k, B_ssm_k, B_ssm_D)
```
